```python
import os as _os
_os.environ.setdefault("JAX_PLATFORMS", "cpu")
import jax
import jax.numpy as jnp

def _softmax(x, axis=-1):
    return jax.nn.softmax(x, axis=axis)
def _gelu(x):
    return jax.nn.gelu(x, approximate=True)
def _silu(x):
    return jax.nn.silu(x)
def _sigmoid(x):
    return jax.nn.sigmoid(x)
def _layernorm(x, axis=-1, eps=1e-5):
    m = jnp.mean(x, axis=axis, keepdims=True)
    v = jnp.var(x, axis=axis, keepdims=True)
    return (x - m) / jnp.sqrt(v + eps)
def _scatter_add(tgt, idx, src, axis=0):
    return tgt.at[idx].add(src)
def _segment_sum(src, seg, n):
    return jax.ops.segment_sum(src, seg, n)
class _Rng:
    def __init__(self, key):
        self._k = key
    def _next(self):
        self._k, sub = jax.random.split(self._k)
        return sub
    def normal(self, shape):
        return jax.random.normal(self._next(), shape, dtype=jnp.bfloat16)
    def randint(self, lo, hi, shape):
        return jax.random.randint(self._next(), shape, lo, hi, dtype=jnp.int32)
    def uniform(self, shape, lo=0.0, hi=1.0):
        return jax.random.uniform(self._next(), shape, jnp.bfloat16, lo, hi)
    def permutation(self, n):
        return jax.random.permutation(self._next(), n)


kernel_name = 'sequential_preLN__mha_block__moe_arch_mod__prompt'

def setup_inputs():
    _rng = _Rng(jax.random.key(int.from_bytes(__import__("os").urandom(4), "little")))
    _w = (lambda a: (lambda t: t.astype(jnp.bfloat16) if jnp.issubdtype(t.dtype, jnp.floating) else t)(jnp.asarray(a)))
    def _A_setup():
        B, S, D, H = 1, 2048, 512, 32
        return {
            "x": _w((lambda *s: _rng.normal(s) * 0.05)(B, S, D)),
            "wqkv": _w((lambda *s: _rng.normal(s) * 0.05)(D, 3 * D)),
            "wo": _w((lambda *s: _rng.normal(s) * 0.05)(D, D)),
        }
    _A_in = _A_setup()

    def _B_setup():
        B, S, D, F, C = 1, 2048, 512, 1792, 2
        return {
            "x": _w((lambda *s: _rng.normal(s) * 0.05)(B, S, D)),
            "w_r": _w((lambda *s: _rng.normal(s) * 0.05)(D)),
            "w_gate": _w((lambda *s: _rng.normal(s) * 0.05)(D, F)),
            "w_up": _w((lambda *s: _rng.normal(s) * 0.05)(D, F)),
            "w_down": _w((lambda *s: _rng.normal(s) * 0.05)(F, D)),
        }
    _B_in = _B_setup()

    return {
        "A_x": _A_in["x"],
        "A_wqkv": _A_in["wqkv"],
        "A_wo": _A_in["wo"],
        "B_x": _B_in["x"],
        "B_w_r": _B_in["w_r"],
        "B_w_gate": _B_in["w_gate"],
        "B_w_up": _B_in["w_up"],
        "B_w_down": _B_in["w_down"],
    }

def reference(A_x, A_wqkv, A_wo, B_x, B_w_r, B_w_gate, B_w_up, B_w_down):
    def _A_ref(x, wqkv, wo):
        B, S, D = x.shape
        H = 32
        Dh = D // H
        qkv = (lambda x, *d: x.transpose(*d))((x @ wqkv).reshape(B, S, 3, H, Dh), 2, 0, 3, 1, 4)
        q, k, v = qkv[0], qkv[1], qkv[2]
        scores = jnp.einsum("bhqd,bhkd->bhqk", q, k) * (Dh ** -0.5)
        p = _softmax(scores, axis=-1)
        o = jnp.einsum("bhqk,bhkd->bhqd", p, v)
        return (lambda x, *d: x.transpose(*d))(o, 0, 2, 1, 3).reshape(B, S, D) @ wo

    def _B_ref(x, w_r, w_gate, w_up, w_down):
        B, S, D = x.shape
        C = 2
        r = x @ w_r
        idx = jnp.argsort(-r, axis=-1)[:, :C]
        idx_e = jnp.repeat(idx.reshape(B, C, 1), D, axis=2)
        x_sel = jnp.take_along_axis(x, idx_e, axis=1)
        g = _silu(x_sel @ w_gate)
        u = x_sel @ w_up
        y = (g * u) @ w_down
        r_sel = _sigmoid(jnp.take_along_axis(r, idx, axis=1))
        y = y * r_sel.reshape(B, C, 1)
        b_off = (jnp.arange(B) * S).reshape(B, 1)
        flat_idx = (idx + b_off).reshape(B * C)
        zero = (x * 0.0).reshape(B * S, D)
        upd = _scatter_add(zero, flat_idx, y.reshape(B * C, D), axis=0)
        return x + upd.reshape(B, S, D)

    x = A_x
    h = x + _A_ref(_layernorm(x, axis=-1), A_wqkv, A_wo)
    h2 = h + _B_ref(_layernorm(h, axis=-1), B_w_r, B_w_gate, B_w_up, B_w_down)
    return h2
```

```python
import math

import jax
import jax.numpy as jnp
from jax import lax
from jax.experimental import pallas as pl
from jax.experimental.pallas import tpu as pltpu

F32 = jnp.float32
BF16 = jnp.bfloat16

S = 2048
D = 512
H = 32
DH = 16
FF = 1792
EPS = 1e-5
QSCALE = (DH ** -0.5) * math.log2(math.e)

BQ = 512
BK = 128
NQB = S // BQ
NKC = S // BK
NI = NQB * NKC
NBLK = BK // 8

L_LO = 2.0 ** -64
L_HI = 2.0 ** 64
F32_MAX = 3.0e38

NT = (((1,), (1,)), ((), ()))
TN = (((0,), (0,)), ((), ()))


def _layernorm(v):
    m = jnp.sum(v, axis=-1, keepdims=True) * (1.0 / D)
    c = v - m
    var = jnp.sum(c * c, axis=-1, keepdims=True) * (1.0 / D)
    return c * lax.rsqrt(var + EPS)


def make_kernel(G=2, HPI=1, ABLK=(256, 256, 512, 512, 512), CBLK=(256,) * 8, NHEAD=H, lchain=0, flags=None,
                skip=""):
    NM = NBLK - G
    a_lo = [sum(ABLK[:i]) for i in range(len(ABLK))]
    c_lo = [sum(CBLK[:i]) for i in range(len(CBLK))]

    def kernel(x_hbm, wqkv_hbm, wo_hbm, wr_ref, wg_hbm, wu_hbm, wd_hbm, out_hbm,
               x_v, wq_v, wk_v, wv_v, wo_v, wg_v, wu_v, wd_v,
               k_v, qt_v, vt_v, ot_v, h_v, out_v,
               ks_v, qm_v, qs_v, lhs_v, kb_v, p_v, acc_v, fin_v,
               x_sem, w_sem, o_sem, f_sem):

        def x_copy(i):
            rows = pl.ds(a_lo[i], ABLK[i])
            return pltpu.make_async_copy(x_hbm.at[0, rows, :], x_v.at[rows, :], x_sem.at[i])

        wq_copy = pltpu.make_async_copy(wqkv_hbm.at[:, pl.ds(0, D)], wq_v, w_sem.at[0])
        wk_copy = pltpu.make_async_copy(wqkv_hbm.at[:, pl.ds(D, D)], wk_v, w_sem.at[1])
        wv_copy = pltpu.make_async_copy(wqkv_hbm.at[:, pl.ds(2 * D, D)], wv_v, w_sem.at[2])
        wo_copy = pltpu.make_async_copy(wo_hbm, wo_v, w_sem.at[3])
        ffn_copies = [
            pltpu.make_async_copy(wg_hbm, wg_v, w_sem.at[4]),
            pltpu.make_async_copy(wu_hbm, wu_v, w_sem.at[5]),
            pltpu.make_async_copy(wd_hbm, wd_v, w_sem.at[6]),
        ]

        lane = lax.broadcasted_iota(jnp.int32, (8, 128), 1)
        sub = lax.broadcasted_iota(jnp.int32, (8, 128), 0)

        def ln1(i):
            return _layernorm(x_v[a_lo[i]:a_lo[i] + ABLK[i], :].astype(F32)).astype(BF16)

        def proj_k(i, xn):
            rows = slice(a_lo[i], a_lo[i] + ABLK[i])
            kk = jnp.dot(xn, wk_v[...], preferred_element_type=F32)
            ks_v[rows, :] = kk[:, 0:128]
            for j in range(1, D // 128):
                k_v[j - 1, rows, :] = kk[:, j * 128:(j + 1) * 128]

        def proj_q(i, xn):
            rows = slice(a_lo[i], a_lo[i] + ABLK[i])
            qq = jnp.dot(xn, wq_v[...], preferred_element_type=F32) * QSCALE
            qt_v[:, rows] = qq.T

        def proj_v(i, xn):
            rows = slice(a_lo[i], a_lo[i] + ABLK[i])
            vv = jnp.dot(xn, wv_v[...], preferred_element_type=F32)
            vt_v[:, rows] = vv.astype(BF16).T

        x_copy(0).start()
        wk_copy.start()
        x_copy(0).wait()
        wq_copy.start()
        xn = ln1(0)
        wk_copy.wait()
        wv_copy.start()
        proj_k(0, xn)
        wq_copy.wait()
        x_copy(1).start()
        proj_q(0, xn)
        wv_copy.wait()
        for i in range(2, len(ABLK)):
            x_copy(i).start()
        x_copy(1).wait()
        xn_next = ln1(1)
        proj_v(0, xn)
        xn = xn_next
        proj_k(1, xn)
        proj_q(1, xn)
        for i in range(2, len(ABLK)):
            x_copy(i).wait()
        wo_copy.start()
        for cp in ffn_copies:
            cp.start()
        proj_v(1, xn)
        for i in range(2, len(ABLK)):
            xn = ln1(i)
            proj_k(i, xn)
            proj_q(i, xn)
            proj_v(i, xn)

        def head_rows(h):
            return pl.ds(pl.multiple_of(h * DH, DH), DH)

        def stage_k(h, s, c, part, nparts, side=False):
            slot = NKC if side else c
            shift = (128 - (h % 8) * DH) % 128
            todo = [("v", j, d) for d in range(DH) for j in range(G)]
            for j in range(NM):
                todo.insert(j * (len(todo) + 1) // NM, ("m", j))
            todo = todo[len(todo) * part // nparts:len(todo) * (part + 1) // nparts]
            base = {}
            for t in todo:
                if t[0] == "m":
                    j = t[1]
                    dst = NM - 1 - j
                    src = ks_v[c * BK + j * 8:c * BK + (j + 1) * 8, :]
                    lhs_v[s][slot][dst * 8:(dst + 1) * 8, :] = pltpu.roll(src, shift, 1)
                else:
                    _, j, d = t
                    if (j, d // 8) not in base:
                        jj = NBLK - 1 - j
                        src = ks_v[c * BK + jj * 8:c * BK + (jj + 1) * 8, :]
                        base[j, d // 8] = jnp.take_along_axis(src, lane % 8 + ((h % 8) * DH + d // 8 * 8), axis=1)
                    b = base[j, d // 8]
                    kb_v[s][slot][d * G + j] = b if d % 8 == 0 else pltpu.roll(b, 128 - d % 8, 1)

        def stage_q(h, s):
            q = qt_v[head_rows(h), :]
            qm_v[s][...] = q
            if G:
                skew = (lane + sub) % 8
                for r in range(DH // 8):
                    for t in range(S // 128):
                        blk = q[r * 8:(r + 1) * 8, t * 128:(t + 1) * 128]
                        qs_v[s][r * 8:(r + 1) * 8, t * 128:(t + 1) * 128] = jnp.take_along_axis(blk, skew, axis=0)

        def mxu_scores(s, c, qb):
            sm = jnp.dot(lhs_v[s][c][:, 0:DH], qm_v[s][:, qb * BQ:(qb + 1) * BQ], preferred_element_type=F32)
            return [sm[j * 8:(j + 1) * 8] for j in range(NM)]

        def vpu_scores(s, c, qb):
            nt = BQ // 128
            acc = [[None] * nt for _ in range(G)]
            for d in range(DH if G else 0):
                kb = [kb_v[s][c][d * G + j] for j in range(G)]
                for t in range(nt):
                    lo = qb * BQ + t * 128
                    q = jnp.broadcast_to(qs_v[s][d:d + 1, lo:lo + 128], (8, 128))
                    for j in range(G):
                        pr = kb[j] * q
                        acc[j][t] = pr if d == 0 else acc[j][t] + pr
            return [jnp.concatenate(a, axis=1) for a in acc]

        def weigh(h, c, qb, blocks):
            p = [jnp.exp2(b) for b in blocks]
            if lchain and c > 0:
                l = acc_v[qb][DH:DH + 8, :]
                for e in p:
                    l = l + e
            else:
                l = p[0]
                for e in p[1:]:
                    l = l + e
                if c > 0:
                    l = acc_v[qb][DH:DH + 8, :] + l
            o = jnp.dot(vt_v[head_rows(h), c * BK:(c + 1) * BK], jnp.concatenate(p[::-1], axis=0),
                        preferred_element_type=F32)
            if c > 0:
                o = acc_v[qb][0:DH, :] + o
            return o, l

        def finalize(h, qb, acc, l, bad):
            lsum = jnp.sum(l, axis=0, keepdims=True)
            o = acc * pltpu.reciprocal(lsum, approx=False)
            ot_v[head_rows(h), qb * BQ:(qb + 1) * BQ] = o.astype(BF16)
            ok = (lsum >= L_LO) & (lsum <= L_HI) & (jnp.abs(o) <= F32_MAX)
            b = jnp.where(ok, 0.0, 1.0)
            b = b[0:8] + b[8:16]
            for t in range(BQ // 128):
                bad = bad + b[:, t * 128:(t + 1) * 128]
            return bad

        for s in range(HPI):
            stage_q(s, s)
            for c in range(NKC):
                stage_k(s, s, c, 0, 1)
        p_v[...] = jnp.zeros(p_v.shape, F32)
        acc_v[NQB - 1][...] = jnp.ones(acc_v[0].shape, F32)
        for qb in range(NQB):
            fin_v[qb][...] = jnp.ones(fin_v[0].shape, F32)

        def head_body(it, bad):
            h0 = it * HPI
            nxt = jnp.minimum(h0 + HPI, H - HPI)

            @pl.when(nxt % 8 == 0)
            def _():
                ks_v[...] = k_v[nxt // 8 - 1]

            prev = [p_v[j * 8:(j + 1) * 8, :] for j in range(NBLK)]
            for i in range(HPI * NI):
                s1, i1 = divmod(i, NI)
                c1, qb1 = divmod(i1, NQB)
                new = vpu_scores(s1, c1, qb1) + mxu_scores(s1, c1, qb1)
                s2, c2 = divmod((s1 * NKC + c1 - 1) % (HPI * NKC), NKC)
                stage_k(nxt + s2, s2, c2, qb1, NQB, side=i < NQB)
                s, i0 = divmod(i - 1, NI)
                c, qb = divmod(i0, NQB)
                h = jnp.maximum(h0 + s, 0)
                o, l = weigh(h, c, qb, prev)
                prev = new
                if c < NKC - 1:
                    acc_v[qb][0:DH, :] = o
                    acc_v[qb][DH:DH + 8, :] = l
                else:
                    fin_v[qb][0:DH, :] = o
                    fin_v[qb][DH:DH + 8, :] = l
                if i1 in (24, 26, 28, 30):
                    q2 = (i1 - 24) // 2
                    bad = finalize(jnp.maximum(h0 + s1 - 1, 0), q2, fin_v[q2][0:DH, :], fin_v[q2][DH:DH + 8, :], bad)
                if i1 == NI - 1:
                    stage_q(nxt + s1, s1)
            for j, b in enumerate(prev):
                p_v[j * 8:(j + 1) * 8, :] = b
            lhs_v[HPI - 1][NKC - 1][...] = lhs_v[HPI - 1][NKC][...]
            if G:
                kb_v[HPI - 1][NKC - 1][...] = kb_v[HPI - 1][NKC][...]
            return bad

        bad = lax.fori_loop(0, NHEAD // HPI, head_body, jnp.zeros((8, 128), F32))
        o, l = weigh(H - 1, NKC - 1, NQB - 1, [p_v[j * 8:(j + 1) * 8, :] for j in range(NBLK)])
        bad = finalize(H - 1, NQB - 1, o, l, bad)
        for qb in range(NQB - 1):
            bad = finalize(H - 1, qb, fin_v[qb][0:DH, :], fin_v[qb][DH:DH + 8, :], bad)

        @pl.when((jnp.sum(bad) != 0.0) & (NHEAD == H))
        def _():
            def safe_head(h, carry):
                @pl.when(h % 8 == 0)
                def _():
                    def krows(i, carry):
                        rows = pl.ds(pl.multiple_of(i * 128, 128), 128)
                        xn = _layernorm(x_v[rows, :].astype(F32)).astype(BF16)
                        cols = pl.ds(pl.multiple_of((h // 8) * 128, 128), 128)
                        ks_v[rows, :] = jnp.dot(xn, wk_v[:, cols], preferred_element_type=F32)
                        return carry
                    lax.fori_loop(0, S // 128, krows, 0)

                def safe_tile(i, carry):
                    cols = pl.ds(pl.multiple_of(i * 128, 128), 128)
                    kk = pltpu.roll(ks_v[...], (128 - (h % 8) * DH) % 128, 1)[:, :DH]
                    sc = jnp.dot(kk, qt_v[head_rows(h), cols], preferred_element_type=F32)
                    p = jnp.exp2(sc - jnp.max(sc, axis=0, keepdims=True))
                    p = p * pltpu.reciprocal(jnp.sum(p, axis=0, keepdims=True), approx=False)
                    o = jnp.dot(vt_v[head_rows(h), :], p.astype(BF16), preferred_element_type=F32)
                    ot_v[head_rows(h), cols] = o.astype(BF16)
                    return carry
                return lax.fori_loop(0, S // 128, safe_tile, carry)
            lax.fori_loop(0, H, safe_head, 0)

        wo_copy.wait()
        for cp in ffn_copies:
            cp.wait()
        wr = wr_ref[...].astype(F32).reshape(1, D)
        r_all = [jnp.zeros((8, 128), F32) for _ in range(S // 1024)]

        def out_copy(i):
            rows = pl.ds(c_lo[i], CBLK[i])
            return pltpu.make_async_copy(out_v.at[rows, :], out_hbm.at[0, rows, :], o_sem.at[i])

        def out_proj(i):
            rows = slice(c_lo[i], c_lo[i] + CBLK[i])
            return lax.dot_general(ot_v[:, rows], wo_v[...], TN, preferred_element_type=F32)

        attn = out_proj(0)
        for i in range(len(CBLK)):
            rows = slice(c_lo[i], c_lo[i] + CBLK[i])
            attn_next = out_proj(i + 1) if i + 1 < len(CBLK) else None
            hh = x_v[rows, :].astype(F32) + attn
            attn = attn_next
            h_v[rows, :] = hh
            ln = _layernorm(hh)
            out_v[rows, :] = (hh + ln).astype(BF16)
            out_copy(i).start()
            r = jnp.sum(ln * wr, axis=-1, keepdims=True)
            for g in range(CBLK[i] // 8):
                gg = c_lo[i] // 8 + g
                r_all[gg // 128] = jnp.where(lane == gg % 128, r[g * 8:(g + 1) * 8], r_all[gg // 128])

        r = jnp.concatenate(r_all, axis=0)
        tok = jnp.concatenate([(lane + 128 * j) * 8 + sub for j in range(S // 1024)], axis=0)
        r = jnp.where(r != r, -jnp.inf, r)
        m1 = jnp.max(r, axis=(0, 1), keepdims=True)
        t1 = jnp.min(jnp.where(r == m1, tok, S - 1), axis=(0, 1), keepdims=True)
        rest = tok != t1
        m2 = jnp.max(jnp.where(rest, r, -jnp.inf), axis=(0, 1), keepdims=True)
        t2 = jnp.min(jnp.where(rest & (r == m2), tok, S - 1), axis=(0, 1), keepdims=True)
        i1 = t1[0, 0]
        i2 = t2[0, 0]

        row = lax.broadcasted_iota(jnp.int32, (16, D), 0)
        h1 = h_v[pl.ds(i1, 1), :]
        h2 = h_v[pl.ds(i2, 1), :]
        hs = jnp.where(row < 8, h1, h2)
        ls = _layernorm(hs)
        rs = jnp.sum(ls * wr, axis=-1, keepdims=True)
        xs = ls.astype(BF16)
        gg = jnp.dot(xs, wg_v[...], preferred_element_type=F32)
        uu = jnp.dot(xs, wu_v[...], preferred_element_type=F32)
        act = (gg * jax.nn.sigmoid(gg) * uu).astype(BF16)
        y = jnp.dot(act, wd_v[...], preferred_element_type=F32) * jax.nn.sigmoid(rs)
        fin = hs + (ls + y)

        for i in range(len(CBLK)):
            out_copy(i).wait()
        b1 = pl.multiple_of((i1 // 16) * 16, 16)
        b2 = pl.multiple_of((i2 // 16) * 16, 16)
        t1v = out_v[pl.ds(b1, 16), :].astype(F32)
        out_v[pl.ds(b1, 16), :] = jnp.where(row == i1 % 16, fin[0:1], t1v).astype(BF16)
        t2v = out_v[pl.ds(b2, 16), :].astype(F32)
        out_v[pl.ds(b2, 16), :] = jnp.where(row == i2 % 16, fin[8:9], t2v).astype(BF16)
        c1 = pltpu.make_async_copy(out_v.at[pl.ds(b1, 16), :], out_hbm.at[0, pl.ds(b1, 16), :], f_sem.at[0])
        c2 = pltpu.make_async_copy(out_v.at[pl.ds(b2, 16), :], out_hbm.at[0, pl.ds(b2, 16), :], f_sem.at[1])
        c1.start()

        @pl.when(b1 != b2)
        def _():
            c2.start()
            c2.wait()

        c1.wait()

    hbm = pl.BlockSpec(memory_space=pltpu.HBM)
    call = pl.pallas_call(
        kernel,
        out_shape=jax.ShapeDtypeStruct((1, S, D), BF16),
        in_specs=[hbm, hbm, hbm, pl.BlockSpec(memory_space=pltpu.VMEM), hbm, hbm, hbm],
        out_specs=hbm,
        scratch_shapes=[
            pltpu.VMEM((S, D), BF16),
            pltpu.VMEM((D, D), BF16),
            pltpu.VMEM((D, D), BF16),
            pltpu.VMEM((D, D), BF16),
            pltpu.VMEM((D, D), BF16),
            pltpu.VMEM((D, FF), BF16),
            pltpu.VMEM((D, FF), BF16),
            pltpu.VMEM((FF, D), BF16),
            pltpu.VMEM((D // 128 - 1, S, 128), F32),
            pltpu.VMEM((D, S), F32),
            pltpu.VMEM((D, S), BF16),
            pltpu.VMEM((D, S), BF16),
            pltpu.VMEM((S, D), F32),
            pltpu.VMEM((S, D), BF16),
            pltpu.VMEM((S, 128), F32),
            [pltpu.VMEM((DH, S), F32)] * HPI,
            [pltpu.VMEM((DH, S), F32)] * HPI,
            [[pltpu.VMEM((NM * 8, 128), F32)] * (NKC + 1)] * HPI,
            [[pltpu.VMEM((max(G, 1) * DH, 8, 128), F32)] * (NKC + 1)] * HPI,
            pltpu.VMEM((BK, BQ), F32),
            [pltpu.VMEM((DH + 8, BQ), F32)] * NQB,
            [pltpu.VMEM((DH + 8, BQ), F32)] * NQB,
            pltpu.SemaphoreType.DMA((len(ABLK),)),
            pltpu.SemaphoreType.DMA((7,)),
            pltpu.SemaphoreType.DMA((len(CBLK),)),
            pltpu.SemaphoreType.DMA((2,)),
        ],
        compiler_params=pltpu.CompilerParams(vmem_limit_bytes=100 * 2 ** 20, flags=flags),
    )

    @jax.jit
    def fn(A_x, A_wqkv, A_wo, B_x, B_w_r, B_w_gate, B_w_up, B_w_down):
        del B_x
        return call(A_x, A_wqkv, A_wo, B_w_r, B_w_gate, B_w_up, B_w_down)

    return fn


def pallas_sequential_preLN__mha_block__moe_arch_mod__prompt_kernel(
        A_x, A_wqkv, A_wo, B_x, B_w_r, B_w_gate, B_w_up, B_w_down):
    return make_kernel(**dict())(A_x, A_wqkv, A_wo, B_x, B_w_r, B_w_gate, B_w_up, B_w_down)
```

```python
import math

import jax
import jax.numpy as jnp
from jax import lax
from jax.experimental import pallas as pl
from jax.experimental.pallas import tpu as pltpu

F32 = jnp.float32
BF16 = jnp.bfloat16

S = 2048
D = 512
H = 32
DH = 16
FF = 1792
EPS = 1e-5
QSCALE = (DH ** -0.5) * math.log2(math.e)

BQ = 512
BK = 128
NQB = S // BQ
NKC = S // BK
NI = NQB * NKC
NBLK = BK // 8
NLT = BQ // 128

L_LO = 2.0 ** -64
L_HI = 2.0 ** 64
F32_MAX = 3.0e38
TINY = 2.0 ** -100

TN = (((0,), (0,)), ((), ()))
NT = (((1,), (1,)), ((), ()))


def _layernorm(v):
    m = jnp.sum(v, axis=-1, keepdims=True) * (1.0 / D)
    c = v - m
    var = jnp.sum(c * c, axis=-1, keepdims=True) * (1.0 / D)
    return c * lax.rsqrt(var + EPS)


def _starts(sizes):
    return [sum(sizes[:i]) for i in range(len(sizes))]


O1 = "w0 L0 wk fk K0 wq w1 fq Q0 L1 K1 L2 Q1 K2 wv w2 late Q2 L3 K3 L4 Q3 K4 L5 Q4 K5 L6 Q5 K6 bases Q6 fv V0 V1 V2 V3 V4 V5 V6"
O2 = "w0 L0 wk fk K0 wq w1 fq Q0 L1 K1 L2 Q1 K2 wv w2 late Q2 fv L3 V0 K3 L4 Q3 K4 L5 Q4 K5 L6 Q5 K6 bases Q6 V1 V2 V3 V4 V5 V6"
O3 = "w0 L0 wk fk L1 K0 K1 wq w1 fq Q0 L2 Q1 K2 L3 Q2 K3 wv w2 late Q3 fv V0 L4 K4 Q4 L5 K5 Q5 L6 K6 Q6 L7 K7 bases Q7 V1 V2 V3 V4 V5 V6 V7"
O4 = "w0 L0 L1 wk fk K0 K1 wq w1 fq Q0 L2 Q1 K2 L3 Q2 K3 wv w2 late Q3 fv V0 L4 K4 Q4 V1 L5 K5 Q5 V2 L6 K6 Q6 L7 K7 bases Q7 V3 V4 V5 V6 V7"
O5 = "w0 L0 wk fk K0 wq fq Q0 w1 wv fv V0 L1 K1 Q1 w2 late V1 L2 K2 Q2 L3 K3 Q3 L4 K4 Q4 L5 K5 Q5 L6 K6 Q6 L7 K7 bases Q7 V2 V3 V4 V5 V6 V7"
O6 = "w0 L0 wk fk K0 wq w1 L1 K1 fq Q0 L2 K2 Q1 wv w2 late Q2 L3 K3 L4 Q3 K4 L5 Q4 K5 L6 Q5 K6 bases Q6 fv V0 V1 V2 V3 V4 V5 V6"
O7 = "w0 L0 wk fk K0 wq w1 fq Q0 L1 K1 wv w2 late Q1 L2 K2 L3 Q2 K3 L4 Q3 K4 L5 Q4 K5 bases Q5 fv V0 V1 V2 V3 V4 V5"
O8 = "w0 L0 wk fk K0 wq w1 fq Q0 L1 K1 L2 Q1 K2 L3 Q2 K3 L4 Q3 K4 wv w2 late Q4 " + " ".join(f"L{i} K{i} Q{i}" for i in range(5, 12)) + " L12 K12 bases Q12 fv " + " ".join(f"V{i}" for i in range(13))
P1 = "w0 L0 wk fk K0 wq w1 fq Q0 L1 K1 L2 Q1 K2 wv w2 late pk Q2 P0 P1 P2 L3 K3 L4 Q3 P3 K4 L5 Q4 P4 K5 L6 Q5 P5 K6 bases Q6 P6 fv V0 V1 V2 V3 V4 V5 V6"


def diag(a, b, n=4):
    return tuple(tuple(b if t == q % n else a for t in range(n)) for q in range(4))


def make_kernel(PAT=(((7, 0),),), HPI=1, ABLK=(512,) + (256,) * 6, XBLK=(512, 512, 1024), order=O1, CBLK=(128,) * 16, OBLK=(1280, 512, 256),
                NHEAD=H, flags=None, skip=False, carryp=True, dmajor=True, fin0=1, fin1=14, mfirst=0, cahead=2,
                stop=0, lchain=1, qend=0, qalt=8, jit=0, malt=False, step=5, PRE=(), smem=True, ctail=256, nochk=True, qnt=False, LP=128, E=1, vf32=False, esave_exp=True):
    VB = [[PAT[c % len(PAT)][qb % len(PAT[c % len(PAT)])] for qb in range(NQB)] for c in range(NKC)]
    VB = [[v if isinstance(v[0], tuple) else (v,) for v in vc] for vc in VB]
    VG = [sorted(set(b for w in VB[c] for v in w for b in v), reverse=True) for c in range(NKC)]
    MG = [[b for b in range(NBLK - 1, -1, -1) if any(b not in v for w in VB[c] for v in w) and (c, b) not in PRE] for c in range(NKC)]
    MG = [[(c, b) for b in MG[c][E if c else 0:]] + ([(c + 1, b) for b in MG[c + 1][:E]] if c + 1 < NKC else [])
          for c in range(NKC)]
    m_at = {cb: n for n, cb in enumerate(cb for m in MG for cb in m)}
    vg_lo = _starts([len(v) for v in VG])
    mg_lo = _starts([len(v) for v in MG])
    NVG = -(-sum(len(v) for v in VG) // 16) * 16
    NMG = sum(len(v) for v in MG)
    x_lo = _starts(XBLK)
    a_lo, c_lo, o_lo = _starts(ABLK), _starts(CBLK), _starts(OBLK)

    def kernel(x_hbm, wqkv_hbm, wo_hbm, wr_ref, wg_hbm, wu_hbm, wd_hbm, out_hbm,
               x_v, wq_v, wk_v, wv_v, wo_v, wg_v, wu_v, wd_v,
               xf_v, wf_v, km_v, kv_v, kp_v, pb_v, pre_v, base_v, qt_v, qk_v, vt_v, ot_v, res_v, ln_v, out_v,
               kms_v, qm_v, qs_v, qa_v, ma_v, lhs_v, kb_v, p_v, early_v, acc_v, fin_v, st_v,
               x_sem, w_sem, o_sem, f_sem):

        def x_copy(i):
            rows = pl.ds(x_lo[i], XBLK[i])
            return pltpu.make_async_copy(x_hbm.at[0, rows, :], x_v.at[rows, :], x_sem.at[i])

        wq_copy = pltpu.make_async_copy(wqkv_hbm.at[:, pl.ds(0, D)], wq_v, w_sem.at[0])
        wk_copy = pltpu.make_async_copy(wqkv_hbm.at[:, pl.ds(D, D)], wk_v, w_sem.at[1])
        wv_copy = pltpu.make_async_copy(wqkv_hbm.at[:, pl.ds(2 * D, D)], wv_v, w_sem.at[2])
        late_copies = [
            pltpu.make_async_copy(wo_hbm, wo_v, w_sem.at[3]),
            pltpu.make_async_copy(wg_hbm, wg_v, w_sem.at[4]),
            pltpu.make_async_copy(wu_hbm, wu_v, w_sem.at[5]),
            pltpu.make_async_copy(wd_hbm, wd_v, w_sem.at[6]),
        ]

        lane = lax.broadcasted_iota(jnp.int32, (8, 128), 1)
        sub = lax.broadcasted_iota(jnp.int32, (8, 128), 0)

        def quadrants(v):
            m, n = v.shape[0] // 2, v.shape[1] // 2
            return v[:m, :n], v[:m, n:], v[m:, :n], v[m:, n:]

        def ln1(i):
            for r in range(0, ABLK[i] // 2, LP):
                top, bot = a_lo[i] + r, a_lo[i] + ABLK[i] // 2 + r
                xx = jnp.concatenate([x_v[top:top + LP, :], x_v[bot:bot + LP, :]], axis=0)
                a11, a12, a21, a22 = quadrants(_layernorm(xx.astype(F32)))
                for n, v in enumerate((a21 + a22, a11 + a12, a11, a22, a11 + a22, a21 - a11, a12 - a22)):
                    xf_v[n, a_lo[i] // 2 + r:a_lo[i] // 2 + r + LP, :] = v.astype(BF16)

        def w_factors(w_v, n, transpose):
            b11, b12, b21, b22 = quadrants(w_v[...].astype(F32))
            for j, v in enumerate((b11, b22, b12 - b22, b21 - b11, b11 + b22, b11 + b12, b21 + b22)):
                v = v.astype(BF16)
                wf_v[n, j] = v.T if transpose else v

        def project(i, n, transpose):
            m = []
            for j in range(7):
                xf = xf_v[j, a_lo[i] // 2:(a_lo[i] + ABLK[i]) // 2, :]
                if transpose:
                    m.append(lax.dot_general(wf_v[n, j], xf, NT, preferred_element_type=F32))
                else:
                    m.append(jnp.dot(xf, wf_v[n, j], preferred_element_type=F32))
            m2, m5, m3, m4, m1, m6, m7 = m
            return (m4 - m5 + m1) + m7, m5 + m3, m2 + m4, (m3 - m2 + m1) + m6

        def project_t(i, n):
            c11, c12, c21, c22 = project(i, n, True)
            return jnp.concatenate([jnp.concatenate([c11, c21], axis=1), jnp.concatenate([c12, c22], axis=1)], axis=0)

        def project_n(i, n):
            c11, c12, c21, c22 = project(i, n, False)
            return jnp.concatenate([jnp.concatenate([c11, c12], axis=1), jnp.concatenate([c21, c22], axis=1)], axis=0)

        def proj_k(i):
            kk = project_n(i, 0)
            for t in range(ABLK[i] // BK):
                c = a_lo[i] // BK + t
                for b in range(NBLK):
                    if (c, b) in m_at:
                        blk = kk[t * BK + b * 8:t * BK + (b + 1) * 8]
                        kms_v[m_at[c, b]] = blk[:, 0:128]
                        for n in range(0 if c <= jit else 1, D // 128):
                            km_v[n, m_at[c, b]] = blk[:, n * 128:(n + 1) * 128]
                for j, (cc, b) in enumerate(PRE):
                    if cc == c:
                        kp_v[j * 8:(j + 1) * 8, :] = kk[t * BK + b * 8:t * BK + (b + 1) * 8]
                for j, b in enumerate(VG[c]):
                    kv_v[(vg_lo[c] + j) * 8:(vg_lo[c] + j + 1) * 8, :] = kk[t * BK + b * 8:t * BK + (b + 1) * 8]

        def proj_q(i):
            qq = project_t(i, 1) * QSCALE if qnt else (project_n(i, 1) * QSCALE).T
            qt_v[:, a_lo[i]:a_lo[i] + ABLK[i]] = qq
            skew = (lane + sub) & 7
            for r in range(D // 8):
                for t in range(ABLK[i] // 128):
                    qk_v[r * 8:(r + 1) * 8, a_lo[i] + t * 128:a_lo[i] + (t + 1) * 128] = jnp.take_along_axis(
                        qq[r * 8:(r + 1) * 8, t * 128:(t + 1) * 128], skew, axis=0)

        def proj_v(i):
            vt_v[:, a_lo[i]:a_lo[i] + ABLK[i]] = project_t(i, 2).astype(vt_v.dtype)

        def k_bases():
            used = vg_lo[-1] + len(VG[-1])
            if used < NVG:
                kv_v[used * 8:, :] = jnp.zeros(((NVG - used) * 8, D), F32)
            kvt = kv_v[...].T
            for r in range(D // 8):
                for n in range(NVG // 16):
                    rep = jnp.concatenate([kvt[r * 8:(r + 1) * 8, n * 128:(n + 1) * 128]] * 16, axis=0).T
                    for j in range(min(16, used - n * 16)):
                        base_v[r // 2, n * 16 + j, r % 2] = rep[j * 8:(j + 1) * 8]

        def pre_keys():
            for j in range(len(PRE)):
                for h in range(H):
                    src = kp_v[j * 8:(j + 1) * 8, (h // 8) * 128:(h // 8 + 1) * 128]
                    for half in range(2):
                        pb_v[h, j, half * 8] = jnp.take_along_axis(src, (lane & 7) + ((h % 8) * DH + half * 8), axis=1)
            for j in range(len(PRE)):
                for h in range(H):
                    for d in range(DH):
                        if d % 8:
                            pb_v[h, j, d] = pltpu.roll(pb_v[h, j, d // 8 * 8], 128 - d % 8, 1)

        def pre_probs(i):
            for h in range(H):
                for t in range(a_lo[i] // 128, (a_lo[i] + ABLK[i]) // 128):
                    acc = [None] * len(PRE)
                    for d in range(DH):
                        q = jnp.broadcast_to(qk_v[h * DH + d:h * DH + d + 1, t * 128:(t + 1) * 128], (8, 128))
                        for j in range(len(PRE)):
                            pr = pb_v[h, j, d] * q
                            acc[j] = pr if d == 0 else acc[j] + pr
                    for j in range(len(PRE)):
                        pre_v[h, j * 8:(j + 1) * 8, t * 128:(t + 1) * 128] = jnp.exp2(acc[j])

        if not skip:
            waits = {"k": wk_copy, "q": wq_copy, "v": wv_copy}
            waits.update({str(i): x_copy(i) for i in range(len(XBLK))})
            steps = order.split()
            for n in steps:
                if n[0] == "w":
                    waits[n[1]].start()
            for n in steps:
                if n[0] == "w":
                    waits[n[1]].wait()
                elif n == "late":
                    for cp in late_copies:
                        cp.start()
                elif n == "pk":
                    pre_keys()
                elif n == "bases":
                    k_bases()
                elif n[0] == "f":
                    ref, idx, tr = {"k": (wk_v, 0, False), "q": (wq_v, 1, qnt), "v": (wv_v, 2, True)}[n[1]]
                    w_factors(ref, idx, tr)
                else:
                    {"P": pre_probs, "L": ln1, "K": proj_k, "Q": proj_q, "V": proj_v}[n[0]](int(n[1:]))

        def head_rows(h):
            return pl.ds(pl.multiple_of(h * DH, DH), DH)

        def to_front(v, h):
            return pltpu.roll(v, (128 - (h & 7) * DH) & 127, 1)

        def stage_k(h, s, c, own=False):
            ng = len(VG[c])
            todo = [(j, d) for d in range(DH) for j in range(ng)] if dmajor else [(j, d) for j in range(ng) for d in range(DH)]
            for r in range(len(MG[c])):
                todo.insert(r if mfirst == 1 else len(todo) if mfirst == 2 else r * (len(todo) + 1) // len(MG[c]), (r,))
            if step < 8:
                todo.sort(key=lambda t: (t[0] * 8 // len(MG[c]) if len(t) == 1 else t[1] % 8))
            done = {}
            for t in todo:
                if len(t) == 1:
                    lhs_v[s][c][t[0] * 8:(t[0] + 1) * 8, :] = to_front(km_v[h >> 3, mg_lo[c] + t[0]] if own else kms_v[mg_lo[c] + t[0]], h)
                else:
                    j, d = t
                    b = base_v[h, vg_lo[c] + j, d // 8]
                    if d % 8 > step:
                        b = pltpu.roll(done[j, d - step], 128 - step, 1)
                    elif d % 8:
                        b = pltpu.roll(b, 128 - d % 8, 1)
                    done[j, d] = b
                    kb_v[s][c][d * ng + j] = b

        def stage_q(h, s):
            qm_v[s][...] = qt_v[head_rows(h), :]
            qs_v[s][...] = qk_v[head_rows(h), :]

        def probs(h, s, c, qb):
            n = NLT // len(VB[c][qb])
            early = {}
            if c > 0:
                for r, (cc, b) in enumerate(MG[c - 1][len(MG[c - 1]) - E:]):
                    early[b] = early_v[qb][r * 8:(r + 1) * 8, :]
            for j, (cc, b) in enumerate(PRE):
                if cc == c:
                    early[b] = pre_v[h, j * 8:(j + 1) * 8, qb * BQ:(qb + 1) * BQ]
            parts = [probs_part(s, c, qb, j * n, n, vb) for j, vb in enumerate(VB[c][qb])]
            return [early[b] if b in early else jnp.concatenate([p[b] for p in parts], axis=1)
                    for b in range(NBLK - 1, -1, -1)]

        def probs_part(s, c, qb, t0, nt, vb):
            sel = [j for j, (cc, b) in enumerate(MG[c]) if cc != c or b not in vb]
            lhs = jnp.concatenate([lhs_v[s][c][j * 8:(j + 1) * 8, 0:DH] for j in sel], axis=0)
            lo = qb * BQ + t0 * 128
            sm = jnp.dot(lhs, qm_v[s][:, lo:lo + nt * 128], preferred_element_type=F32)
            by_blk = {}
            n = 0
            for r, j in enumerate(sel):
                cc, b = MG[c][j]
                e = jnp.exp2(sm[r * 8:(r + 1) * 8])
                if cc == c:
                    by_blk[b] = e
                else:
                    early_v[qb][n * 8:(n + 1) * 8, t0 * 128:(t0 + nt) * 128] = e
                    n += 1
            acc = {}
            for d in range(DH):
                for t in range(nt):
                    q = (qa_v if c >= NKC - qalt else qs_v)[s][d:d + 1, lo + t * 128:lo + (t + 1) * 128]
                    q = jnp.broadcast_to(q, (8, 128))
                    for b in vb:
                        pr = kb_v[s][c][d * len(VG[c]) + VG[c].index(b)] * q
                        acc[b, t] = pr if d == 0 else acc[b, t] + pr
            for b in vb:
                by_blk[b] = jnp.exp2(jnp.concatenate([acc[b, t] for t in range(nt)], axis=1))
            return by_blk

        def swap_at(qb, t):
            return fin0 + ((t * NQB + qb) * (fin1 - fin0)) // (NQB * NLT - 1)

        def slot(c, qb, t):
            return (fin_v if c >= swap_at(qb, t) else acc_v)[qb]

        def weigh(h, c, qb, p):
            o = jnp.dot(vt_v[head_rows(h), c * BK:(c + 1) * BK], jnp.concatenate(p[::-1], axis=0),
                        preferred_element_type=F32)
            out = []
            for t in range(NLT):
                cols = slice(t * 128, (t + 1) * 128)
                ot = o[:, cols]
                terms = [e[:, cols] for e in p]
                if c > 0:
                    ot = slot(c - 1, qb, t)[0:DH, cols] + ot
                    old = slot(c - 1, qb, t)[DH:DH + 8, cols]
                    terms = [old] + terms if lchain else terms + [old]
                l = terms[0]
                for e in terms[1:]:
                    l = l + e
                out.append((ot, l))
            return out

        def finalize(h, qb, t, acc, l, stats):
            lsum = jnp.sum(l, axis=0, keepdims=True)
            r = pltpu.reciprocal(lsum, approx=True)
            o = acc * (r * (2.0 - lsum * r))
            lo = qb * BQ + t * 128
            ot_v[head_rows(h), lo:lo + 128] = o.astype(BF16)
            if smem:
                n = qb * NLT + t
                st_v[n, 0, 0:1] = jnp.minimum(st_v[n, 0, 0:1], lsum)
                st_v[n, 1, 0:1] = jnp.maximum(st_v[n, 1, 0:1], lsum)
                st_v[n, 2] = st_v[n, 2] + o[0:8] + o[8:16]
                return stats
            return jnp.minimum(stats[0], lsum), jnp.maximum(stats[1], lsum), stats[2] + o[0:8] + o[8:16]

        def finalize_stored(h, qb, t, stats):
            cols = slice(t * 128, (t + 1) * 128)
            return finalize(h, qb, t, fin_v[qb][0:DH, cols], fin_v[qb][DH:DH + 8, cols], stats)

        for s in range(0 if skip else HPI):
            for c in range((jit if s == 0 else 0) if jit else NKC):
                stage_k(s, s, c)
            stage_q(s, s)
        p_v[...] = jnp.zeros(p_v.shape, F32)
        for qb in range(NQB):
            fin_v[qb][...] = jnp.ones(fin_v[0].shape, F32)

        def carried():
            p = [p_v[j * 8:(j + 1) * 8, :] for j in range(NBLK)]
            return p

        def head_body(it, stats):
            h0 = it * HPI
            nxt = jnp.minimum(h0 + HPI, H - HPI)

            cur_h = h0 if jit else nxt

            @pl.when((cur_h & 7 == 0) & (cur_h > 0))
            def _():
                kms_v[...] = km_v[cur_h >> 3]

            prev = carried()
            for i in range(HPI * NI):
                s1, i1 = divmod(i, NI)
                c1, qb1 = divmod(i1, NQB)
                new = probs(h0 + s1, s1, c1, qb1)
                s, i0 = divmod(i - 1, NI)
                c, qb = divmod(i0, NQB)
                sums = weigh(jnp.maximum(h0 + s, 0), c, qb, prev)
                if jit:
                    if qb1 == 0:
                        s2, c2 = divmod(s1 * NKC + c1 + jit, NKC)
                        if s2 < HPI:
                            stage_k(h0 + s2, s2, c2)
                        else:
                            stage_k(nxt, 0, c2, own=True)
                elif qb1 == NQB - 1:
                    stage_k(nxt + s1, s1, c1)
                prev = new
                for t, (o, l) in enumerate(sums):
                    if c == swap_at(qb, t):
                        stats = finalize_stored(jnp.maximum(h0 + s - 1, 0), qb, t, stats)
                    slot(c, qb, t)[0:DH, t * 128:(t + 1) * 128] = o
                    slot(c, qb, t)[DH:DH + 8, t * 128:(t + 1) * 128] = l
                if i1 == (qend if qend else NI - 1) and (not qend or s1 > 0):
                    stage_q(nxt + s1 - (1 if qend else 0), s1 - (1 if qend else 0))
                if qend and i == HPI * NI - 1:
                    stage_q(nxt + s1, s1)
                if qalt and i1 == 8:
                    qa_v[s1][...] = qs_v[s1][...]
                    if malt:
                        ma_v[s1][...] = qm_v[s1][...]
            for j, b in enumerate(prev):
                p_v[j * 8:(j + 1) * 8, :] = b
            return stats

        if stop == 1:
            for cp in late_copies:
                cp.wait()
            return
        one = jnp.ones((1, 128), F32)
        st_v[...] = jnp.ones(st_v.shape, F32)
        stats = lax.fori_loop(0, NHEAD // HPI, head_body, 0 if smem else (one, one, jnp.zeros((8, 128), F32)))
        for t, (o, l) in enumerate(weigh(H - 1, NKC - 1, NQB - 1, carried())):
            stats = finalize(H - 1, NQB - 1, t, o, l, stats)
            for qb in range(NQB - 1):
                stats = finalize_stored(H - 1, qb, t, stats)
        if smem:
            stats = (jnp.min(st_v[:, 0], axis=0), jnp.max(st_v[:, 1], axis=0), jnp.sum(st_v[:, 2], axis=0))
        bad = jnp.where((stats[0] >= L_LO) & (stats[1] <= L_HI) & (jnp.abs(stats[2]) <= F32_MAX), 0.0, 1.0)

        if skip:
            res_v[0:8, 0:128] = bad
            pltpu.sync_copy(out_v, out_hbm.at[0])
            return

        @pl.when((jnp.sum(bad) != 0.0) & (NHEAD == H))
        def _():
            def k_rows(i, carry):
                rows = pl.ds(pl.multiple_of(i * 128, 128), 128)
                xn = _layernorm(x_v[rows, :].astype(F32)).astype(BF16)
                res_v[rows, :] = jnp.dot(xn, wk_v[...], preferred_element_type=F32)
                return carry
            lax.fori_loop(0, S // 128, k_rows, 0)

            def safe_tile(i, carry):
                h = i // (S // 128)
                cols = pl.ds(pl.multiple_of((i % (S // 128)) * 128, 128), 128)
                kk = to_front(res_v[:, pl.ds(pl.multiple_of((h // 8) * 128, 128), 128)], h)[:, :DH]
                sc = jnp.dot(kk, qt_v[head_rows(h), cols], preferred_element_type=F32)
                p = jnp.exp2(sc - jnp.max(sc, axis=0, keepdims=True))
                p = p * pltpu.reciprocal(jnp.sum(p, axis=0, keepdims=True), approx=False)
                o = jnp.dot(vt_v[head_rows(h), :], p.astype(BF16), preferred_element_type=F32)
                ot_v[head_rows(h), cols] = o.astype(BF16)
                return carry
            lax.fori_loop(0, H * (S // 128), safe_tile, 0)

        for cp in late_copies:
            cp.wait()
        wr = wr_ref[...].astype(F32).reshape(1, D)

        def out_copy(i):
            rows = pl.ds(o_lo[i], OBLK[i])
            return pltpu.make_async_copy(out_v.at[rows, :], out_hbm.at[0, rows, :], o_sem.at[i])

        def residual(i):
            rows = slice(c_lo[i], c_lo[i] + CBLK[i])
            return x_v[rows, :].astype(F32) + lax.dot_general(ot_v[:, rows], wo_v[...], TN, preferred_element_type=F32)

        def router_key(r, tok):
            r = jnp.clip(r + TINY, -F32_MAX, F32_MAX)
            return pltpu.bitcast((pltpu.bitcast(r, jnp.int32) | (S - 1)) ^ tok, F32)

        packed = [jnp.full((8, 128), -F32_MAX, F32) for _ in range(S // 1024)]
        tail_keys = []
        pend = [residual(i) for i in range(cahead)]
        for i in range(len(CBLK)):
            rows = slice(c_lo[i], c_lo[i] + CBLK[i])
            if i + cahead < len(CBLK):
                pend.append(residual(i + cahead))
            hh = pend.pop(0)
            ln = _layernorm(hh)
            r = jnp.sum(ln * wr, axis=-1, keepdims=True)
            res = hh + ln
            ln_v[rows, :] = ln
            res_v[rows, :] = res
            out_v[rows, :] = res.astype(BF16)
            for j in range(len(OBLK)):
                if o_lo[j] + OBLK[j] == c_lo[i] + CBLK[i]:
                    out_copy(j).start()
            for n in range(CBLK[i] // 8):
                g = c_lo[i] // 8 + n
                rg = r[n * 8:(n + 1) * 8]
                if g * 8 < S - ctail:
                    packed[g // 128] = jnp.where(lane == g % 128, rg, packed[g // 128])
                else:
                    tail_keys.append(router_key(rg, sub[:, 0:1] + g * 8))

        keys = [router_key(v, (lane + 128 * j) * 8 + sub) for j, v in enumerate(packed)]
        top1 = jnp.max(jnp.maximum(keys[0], keys[1]), axis=1, keepdims=True)
        keys = [jnp.where(k == top1, -jnp.inf, k) for k in keys]
        top2 = jnp.max(jnp.maximum(keys[0], keys[1]), axis=1, keepdims=True)
        for key in tail_keys:
            top2 = jnp.maximum(top2, jnp.minimum(top1, key))
            top1 = jnp.maximum(top1, key)
        for w in (4, 2, 1):
            o1, o2 = pltpu.roll(top1, w, 0), pltpu.roll(top2, w, 0)
            top2 = jnp.maximum(jnp.maximum(top2, o2), jnp.minimum(top1, o1))
            top1 = jnp.maximum(top1, o1)

        def token(key):
            return (~pltpu.bitcast(key, jnp.int32) & (S - 1))[0, 0]

        i1 = token(top1)
        i2 = token(top2)
        row = lax.broadcasted_iota(jnp.int32, (16, D), 0)
        xs = jnp.where(row < 8, ln_v[pl.ds(i1, 1), :], ln_v[pl.ds(i2, 1), :])
        hs = jnp.where(row < 8, res_v[pl.ds(i1, 1), :], res_v[pl.ds(i2, 1), :])
        rs = jnp.sum(xs * wr, axis=-1, keepdims=True)
        xs = xs.astype(BF16)
        gg = jnp.dot(xs, wg_v[...], preferred_element_type=F32)
        uu = jnp.dot(xs, wu_v[...], preferred_element_type=F32)
        act = (gg * jax.nn.sigmoid(gg) * uu).astype(BF16)
        fin = hs + jnp.dot(act, wd_v[...], preferred_element_type=F32) * jax.nn.sigmoid(rs)

        for i in range(len(OBLK)):
            out_copy(i).wait()
        b1 = pl.multiple_of((i1 >> 4) * 16, 16)
        b2 = pl.multiple_of((i2 >> 4) * 16, 16)
        t1v = out_v[pl.ds(b1, 16), :].astype(F32)
        out_v[pl.ds(b1, 16), :] = jnp.where(row == i1 & 15, fin[0:1], t1v).astype(BF16)
        t2v = out_v[pl.ds(b2, 16), :].astype(F32)
        out_v[pl.ds(b2, 16), :] = jnp.where(row == i2 & 15, fin[8:9], t2v).astype(BF16)
        c1 = pltpu.make_async_copy(out_v.at[pl.ds(b1, 16), :], out_hbm.at[0, pl.ds(b1, 16), :], f_sem.at[0])
        c2 = pltpu.make_async_copy(out_v.at[pl.ds(b2, 16), :], out_hbm.at[0, pl.ds(b2, 16), :], f_sem.at[1])
        c1.start()

        @pl.when(b1 != b2)
        def _():
            c2.start()
            c2.wait()

        c1.wait()

    hbm = pl.BlockSpec(memory_space=pltpu.HBM)
    call = pl.pallas_call(
        kernel,
        out_shape=jax.ShapeDtypeStruct((1, S, D), BF16),
        in_specs=[hbm, hbm, hbm, pl.BlockSpec(memory_space=pltpu.VMEM), hbm, hbm, hbm],
        out_specs=hbm,
        scratch_shapes=[
            pltpu.VMEM((S, D), BF16),
            pltpu.VMEM((D, D), BF16),
            pltpu.VMEM((D, D), BF16),
            pltpu.VMEM((D, D), BF16),
            pltpu.VMEM((D, D), BF16),
            pltpu.VMEM((D, FF), BF16),
            pltpu.VMEM((D, FF), BF16),
            pltpu.VMEM((FF, D), BF16),
            pltpu.VMEM((7, S // 2, D // 2), BF16),
            pltpu.VMEM((3, 7, D // 2, D // 2), BF16),
            pltpu.VMEM((D // 128, NMG, 8, 128), F32),
            pltpu.VMEM((NVG * 8, D), F32),
            pltpu.VMEM((max(len(PRE), 1) * 8, D), F32),
            pltpu.VMEM((H, max(len(PRE), 1), DH, 8, 128), F32),
            pltpu.VMEM((H, max(len(PRE), 1) * 8, S), F32),
            pltpu.VMEM((H, NVG, 2, 8, 128), F32),
            pltpu.VMEM((D, S), F32),
            pltpu.VMEM((D, S), F32),
            pltpu.VMEM((D, S), F32 if vf32 else BF16),
            pltpu.VMEM((D, S), BF16),
            pltpu.VMEM((S, D), F32),
            pltpu.VMEM((S, D), F32),
            pltpu.VMEM((S, D), BF16),
            pltpu.VMEM((NMG, 8, 128), F32),
            [pltpu.VMEM((DH, S), F32)] * HPI,
            [pltpu.VMEM((DH, S), F32)] * HPI,
            [pltpu.VMEM((DH, S), F32)] * HPI,
            [pltpu.VMEM((DH, S), F32)] * HPI,
            [[pltpu.VMEM((BK, 128), F32) for m in MG]] * HPI,
            [[pltpu.VMEM((len(v) * DH, 8, 128), F32) for v in VG]] * HPI,
            pltpu.VMEM((BK, BQ), F32),
            [pltpu.VMEM((max(E, 1) * 8, BQ), F32)] * NQB,
            [pltpu.VMEM((DH + 8, BQ), F32)] * NQB,
            [pltpu.VMEM((DH + 8, BQ), F32)] * NQB,
            pltpu.VMEM((NQB * NLT, 3, 8, 128), F32),
            pltpu.SemaphoreType.DMA((len(XBLK),)),
            pltpu.SemaphoreType.DMA((7,)),
            pltpu.SemaphoreType.DMA((len(OBLK),)),
            pltpu.SemaphoreType.DMA((2,)),
        ],
        compiler_params=pltpu.CompilerParams(vmem_limit_bytes=110 * 2 ** 20, flags=flags,
                                              disable_bounds_checks=nochk, disable_semaphore_checks=nochk),
    )

    @jax.jit
    def fn(A_x, A_wqkv, A_wo, B_x, B_w_r, B_w_gate, B_w_up, B_w_down):
        del B_x
        return call(A_x, A_wqkv, A_wo, B_w_r, B_w_gate, B_w_up, B_w_down)

    return fn


def pallas_sequential_preLN__mha_block__moe_arch_mod__prompt_kernel(
        A_x, A_wqkv, A_wo, B_x, B_w_r, B_w_gate, B_w_up, B_w_down):
    return make_kernel(**dict())(A_x, A_wqkv, A_wo, B_x, B_w_r, B_w_gate, B_w_up, B_w_down)
```

```python
import math

import jax
import jax.numpy as jnp
from jax import lax
from jax.experimental import pallas as pl
from jax.experimental.pallas import tpu as pltpu

F32 = jnp.float32
BF16 = jnp.bfloat16
U32 = jnp.uint32

S = 2048
D = 512
H = 32
DH = 16
FF = 1792
EPS = 1e-5
QSCALE = DH ** -0.5 * math.log2(math.e)

BK = 128
BQ = 512
NKC = S // BK
NQB = S // BQ
NBLK = BK // 8
NLT = BQ // 128

VPU_FIXED = [0, 7]
VPU_EXTRA = 12
EXTRA_TILES = ([["0000"] * 4] + [["1000", "0100", "0010", "0001"]] * 2
               + [["1100", "0011", "1100", "0011"]] * 12 + [["1000", "0100", "0010", "0001"]])
VPU_BLOCKS = [VPU_FIXED + ([VPU_EXTRA] if "1" in "".join(x) else []) for x in EXTRA_TILES]
MXU_BLOCKS = [b for b in range(NBLK - 1, -1, -1) if b not in VPU_FIXED]
NM = len(MXU_BLOCKS)
EARLY = 2
NEW_SUMS = 1
LATE_Q = NKC - 4

PROJ_ORDER = ("w0 L0 wk fk K0 wq w1 fq L2 Q0 L1 K2 K1 wv w2 late Q1 L3 Q2 K3 Q3 L4 K4 B0 L5 K5 Q4 L6 fv "
              "Q6 Q5 K6 V3 B1 B2 V1 V0 V2 V4 V6 V5").split()
X_ROWS = [512, 512, 1024]
PROJ_ROWS = [512] + [256] * 6
OUT_ROWS = [1280, 512, 256]
RES_ROWS = 128

SUM_LO = 2.0 ** -80
SUM_HI = 2.0 ** 120
F32_MAX = 3.0e38
TINY = 2.0 ** -100

TN = (((0,), (0,)), ((), ()))
NT = (((1,), (1,)), ((), ()))


def _starts(sizes):
    return [sum(sizes[:i]) for i in range(len(sizes))]


X_LO, PROJ_LO, OUT_LO = _starts(X_ROWS), _starts(PROJ_ROWS), _starts(OUT_ROWS)
VPU_LO = _starts([8 * len(v) for v in VPU_BLOCKS])
VPU_KEYS = VPU_LO[-1] + 8 * len(VPU_BLOCKS[-1])
VPU_KEYS_PAD = -(-VPU_KEYS // 128) * 128
MXU_KEYS = NKC * NM * 8


def _mxu_row(c, b):
    return (c * NM + MXU_BLOCKS.index(b) - EARLY) * 8 % MXU_KEYS


def _center(v):
    c = v - jnp.sum(v, axis=-1, keepdims=True) * (1.0 / D)
    return c, lax.rsqrt(jnp.sum(c * c, axis=-1, keepdims=True) * (1.0 / D) + EPS)


def _layernorm(v):
    c, rstd = _center(v)
    return c * rstd


def _pack(v):
    return pltpu.bitcast(v.astype(BF16), U32)


def _unpack(v):
    return pltpu.bitcast(v, BF16)


def _quadrants(v):
    m, n = v.shape[0] // 2, v.shape[1] // 2
    return v[:m, :n], v[:m, n:], v[m:, :n], v[m:, n:]


def _blocks(v):
    return [v[r:r + 8] for r in range(0, v.shape[0], 8)]


def _head_rows(h):
    return pl.ds(pl.multiple_of(h * DH, DH), DH)


def _head_pairs(h):
    return pl.ds(pl.multiple_of(h * (DH // 2), DH // 2), DH // 2)


def _to_front(v, h):
    return pltpu.roll(v, (128 - (h & 7) * DH) & 127, 1)


def _router_key(r, tok):
    r = jnp.clip(r + TINY, -F32_MAX, F32_MAX)
    return pltpu.bitcast((pltpu.bitcast(r, jnp.int32) | (S - 1)) ^ tok, F32)


def _kernel(x_hbm, wqkv_hbm, wo_hbm, wr_ref, wg_hbm, wu_hbm, wd_hbm, out_hbm,
            x_v, wq_v, wk_v, wv_v, wo_v, wg_v, wu_v, wd_v,
            xf_v, wf_v, km_v, kv_v, base_v, qt_v, qk_v, vt_v, ot_v, res_v, ln_v, out_v,
            kms_v, qm_v, qs_v, qa_v, lhs_v, kb_v, p_v, early_v, acc_v, fin_v, st_v, idx_s,
            x_sem, w_sem, o_sem, f_sem):
    lane = lax.broadcasted_iota(jnp.int32, (8, 128), 1)
    sub = lax.broadcasted_iota(jnp.int32, (8, 128), 0)

    first_copies = {
        "q": pltpu.make_async_copy(wqkv_hbm.at[:, pl.ds(0, D)], wq_v, w_sem.at[0]),
        "k": pltpu.make_async_copy(wqkv_hbm.at[:, pl.ds(D, D)], wk_v, w_sem.at[1]),
        "v": pltpu.make_async_copy(wqkv_hbm.at[:, pl.ds(2 * D, D)], wv_v, w_sem.at[2]),
    }
    for i, (lo, n) in enumerate(zip(X_LO, X_ROWS)):
        first_copies[str(i)] = pltpu.make_async_copy(
            x_hbm.at[0, pl.ds(lo, n), :], x_v.at[pl.ds(lo, n), :], x_sem.at[i])
    late_copies = [
        pltpu.make_async_copy(wo_hbm, wo_v, w_sem.at[3]),
        pltpu.make_async_copy(wg_hbm, wg_v, w_sem.at[4]),
        pltpu.make_async_copy(wu_hbm, wu_v, w_sem.at[5]),
        pltpu.make_async_copy(wd_hbm, wd_v, w_sem.at[6]),
    ]
    out_copies = [
        pltpu.make_async_copy(out_v.at[pl.ds(lo, n), :], out_hbm.at[0, pl.ds(lo, n), :], o_sem.at[i])
        for i, (lo, n) in enumerate(zip(OUT_LO, OUT_ROWS))
    ]

    def ln1(i):
        half = PROJ_ROWS[i] // 2
        for r in range(0, half, 128):
            top, bot = PROJ_LO[i] + r, PROJ_LO[i] + half + r
            xx = jnp.concatenate([x_v[top:top + 128, :], x_v[bot:bot + 128, :]], axis=0)
            a11, a12, a21, a22 = _quadrants(_layernorm(xx.astype(F32)))
            lo = (PROJ_LO[i] // 2 + r) // 2
            for n, v in enumerate((a21 + a22, a11 + a12, a11, a22, a11 + a22, a21 - a11, a12 - a22)):
                xf_v[n, lo:lo + 64, :] = _pack(v)

    def w_factors(name):
        w_v, n = {"k": (wk_v, 0), "q": (wq_v, 1), "v": (wv_v, 2)}[name]
        b11, b12, b21, b22 = _quadrants(w_v[...].astype(F32))
        for j, v in enumerate((b11, b22, b12 - b22, b21 - b11, b11 + b22, b11 + b12, b21 + b22)):
            wf_v[n, j] = _pack(v.T if name == "v" else v)

    def project(i, n, transpose):
        m = []
        for j in range(7):
            xf = _unpack(xf_v[j, PROJ_LO[i] // 4:(PROJ_LO[i] + PROJ_ROWS[i]) // 4, :])
            wf = _unpack(wf_v[n, j])
            if transpose:
                m.append(lax.dot_general(wf, xf, NT, preferred_element_type=F32))
            else:
                m.append(jnp.dot(xf, wf, preferred_element_type=F32))
        m2, m5, m3, m4, m1, m6, m7 = m
        c11, c12, c21, c22 = (m4 - m5 + m1) + m7, m5 + m3, m2 + m4, (m3 - m2 + m1) + m6
        if transpose:
            c12, c21 = c21, c12
        return jnp.concatenate([jnp.concatenate([c11, c12], axis=1), jnp.concatenate([c21, c22], axis=1)], axis=0)

    def proj_k(i):
        kk = _blocks(project(i, 0, False))
        for t in range(PROJ_ROWS[i] // BK):
            c = PROJ_LO[i] // BK + t
            for part in (MXU_BLOCKS[:EARLY], MXU_BLOCKS[EARLY:]):
                v = jnp.concatenate([kk[t * NBLK + b] for b in part], axis=0)
                rows = slice(_mxu_row(c, part[0]), _mxu_row(c, part[0]) + v.shape[0])
                kms_v[rows, :] = v[:, 0:128]
                for n in range(0 if c == 0 else 1, D // 128):
                    km_v[n, rows, :] = v[:, n * 128:(n + 1) * 128]
            v = jnp.concatenate([kk[t * NBLK + b] for b in VPU_BLOCKS[c]], axis=0)
            kv_v[VPU_LO[c]:VPU_LO[c] + v.shape[0], :] = v

    def proj_q(i):
        qq = (project(i, 1, False) * QSCALE).T
        qt_v[:, PROJ_LO[i]:PROJ_LO[i] + PROJ_ROWS[i]] = qq
        skew = (lane + sub) & 7
        for t in range(0, PROJ_ROWS[i], 128):
            tile = [jnp.take_along_axis(b, skew, axis=0) for b in _blocks(qq[:, t:t + 128])]
            qk_v[:, PROJ_LO[i] + t:PROJ_LO[i] + t + 128] = jnp.concatenate(tile, axis=0)

    def proj_v(i):
        vt_v[:, PROJ_LO[i]:PROJ_LO[i] + PROJ_ROWS[i]] = _pack(project(i, 2, True))

    def k_bases(n):
        if (n + 1) * 128 > VPU_KEYS:
            kv_v[VPU_KEYS:, :] = jnp.zeros((VPU_KEYS_PAD - VPU_KEYS, D), F32)
        for r, b in enumerate(_blocks(kv_v[n * 128:(n + 1) * 128, :].T)):
            base_v[r // 2, r % 2, n * 128:(n + 1) * 128, :] = jnp.concatenate([b] * 16, axis=0).T

    for n in PROJ_ORDER:
        if n[0] == "w":
            first_copies[n[1]].start()
    for n in PROJ_ORDER:
        if n == "late":
            for cp in late_copies:
                cp.start()
        elif n[0] == "w":
            first_copies[n[1]].wait()
        elif n[0] == "f":
            w_factors(n[1])
        else:
            {"L": ln1, "K": proj_k, "Q": proj_q, "V": proj_v, "B": k_bases}[n[0]](int(n[1]))

    def stage_keys(h, c, step):
        own = NM - EARLY if c == NKC - 1 else NM
        rows = slice(VPU_LO[c], VPU_LO[c] + 8 * len(VPU_BLOCKS[c]))
        turns = [jnp.concatenate([base_v[h, 0, rows, :], base_v[h, 1, rows, :]], axis=0)]
        for r in range(8):
            if r > step:
                turns.append(pltpu.roll(turns[r - step], 128 - step, 1))
            elif r:
                turns.append(pltpu.roll(turns[0], 128 - r, 1))
            if r < 7:
                lo, hi = own * r // 7 * 8, own * (r + 1) // 7 * 8
                lhs_v[c][lo:hi, :] = _to_front(kms_v[c * NM * 8 + lo:c * NM * 8 + hi, :], h)
        if own < NM:
            h2 = jnp.minimum(h + 1, H - 1)
            lhs_v[c][own * 8:NM * 8, :] = _to_front(km_v[h2 >> 3, MXU_KEYS - EARLY * 8:, :], h2)
        kb_v[c][...] = jnp.concatenate(turns, axis=0)

    def probs(c, qb):
        by_blk = dict(zip(MXU_BLOCKS[:EARLY], _blocks(early_v[qb][...])))
        lhs = _blocks(lhs_v[c][0:NM * 8, 0:DH])
        q_v = qa_v if c >= LATE_Q else qs_v
        last = c == NKC - 1
        tiles = []
        for t in range(NLT):
            cols = slice(qb * BQ + t * 128, qb * BQ + (t + 1) * 128)
            on_vpu = VPU_FIXED + ([VPU_EXTRA] if EXTRA_TILES[c][qb][t] == "1" else [])
            names = MXU_BLOCKS[EARLY:] + ([] if last else [None] * EARLY)
            take = [j for j, b in enumerate(names) if b not in on_vpu]
            e = jnp.exp2(jnp.dot(jnp.concatenate([lhs[j] for j in take], axis=0), qm_v[0:DH, cols],
                                 preferred_element_type=F32))
            tile = {names[j]: v for j, v in zip(take, _blocks(e)) if names[j] is not None}
            if not last:
                early_v[qb][:, t * 128:(t + 1) * 128] = e[-EARLY * 8:]
            s = None
            for d in range(DH):
                lo = (d % 8 * 2 + d // 8) * len(VPU_BLOCKS[c]) * 8
                term = kb_v[c][lo:lo + len(on_vpu) * 8, :] * q_v[d:d + 1, cols]
                s = term if d == 0 else s + term
            tile.update(zip(on_vpu, _blocks(jnp.exp2(s))))
            tiles.append(tile)
        if last:
            early_v[qb][...] = jnp.exp2(jnp.dot(
                jnp.concatenate(lhs[-EARLY:], axis=0), qm_v[DH:2 * DH, qb * BQ:(qb + 1) * BQ],
                preferred_element_type=F32))
        by_blk.update({b: jnp.concatenate([tile[b] for tile in tiles], axis=1) for b in tiles[0]})
        return [by_blk[b] for b in range(NBLK - 1, -1, -1)]

    def sums_after(c):
        return fin_v if c >= NEW_SUMS else acc_v

    def weigh(h, c, qb, p):
        o = jnp.dot(_unpack(vt_v[_head_pairs(h), c * BK:(c + 1) * BK]), jnp.concatenate(p[::-1], axis=0),
                    preferred_element_type=F32)
        terms = p[2:12] + [p[1]] + p[12:] + [p[0]]
        if c > 0:
            old = sums_after(c - 1)[qb][...]
            o = old[0:DH] + o
            terms.append(old[DH:])
        l = terms[0]
        for v in terms[1:]:
            l = l + v
        return jnp.concatenate([o, l], axis=0)

    def finalize(h, qb, sums):
        l = jnp.sum(sums[DH:], axis=0, keepdims=True)
        r = pltpu.reciprocal(l, approx=True)
        o = sums[0:DH] * (r * (2.0 - l * r))
        cols = slice(qb * BQ, (qb + 1) * BQ)
        ot_v[_head_pairs(h), cols] = _pack(o)
        st_v[0, 0:1, cols] = jnp.minimum(st_v[0, 0:1, cols], l)
        st_v[1, 0:1, cols] = jnp.maximum(st_v[1, 0:1, cols], l)
        st_v[2, :, cols] = st_v[2, :, cols] + o[0:8] + o[8:16]

    for c in range(NKC):
        stage_keys(0, c, 8)
    qm_v[0:DH, :] = qt_v[0:DH, :]
    qs_v[...] = qk_v[0:DH, :]
    first = jnp.exp2(jnp.dot(kms_v[MXU_KEYS - EARLY * 8:, 0:DH], qt_v[0:DH, :], preferred_element_type=F32))
    for qb in range(NQB):
        early_v[qb][...] = first[:, qb * BQ:(qb + 1) * BQ]
    p_v[...] = jnp.zeros(p_v.shape, F32)
    for ref in (*fin_v, st_v):
        ref[...] = jnp.ones(ref.shape, F32)

    def head_body(h, carry):
        prv = jnp.maximum(h - 1, 0)
        nxt = jnp.minimum(h + 1, H - 1)

        @pl.when(nxt & 7 == 0)
        def _():
            kms_v[...] = km_v[nxt >> 3]

        p, (ph, pc, pq) = _blocks(p_v[...]), (prv, NKC - 1, NQB - 1)
        for c in range(NKC):
            for qb in range(NQB):
                p_next = probs(c, qb)
                sums = weigh(ph, pc, pq, p)
                if pc == NEW_SUMS:
                    finalize(prv, pq, fin_v[pq][...])
                sums_after(pc)[pq][...] = sums
                p, (ph, pc, pq) = p_next, (h, c, qb)
            stage_keys(nxt, c, 2)
            if c == 1:
                qa_v[...] = qs_v[...]
                qm_v[DH:2 * DH, :] = qt_v[_head_rows(nxt), :]
        qm_v[0:DH, :] = qm_v[DH:2 * DH, :]
        qs_v[...] = qk_v[_head_rows(nxt), :]
        p_v[...] = jnp.concatenate(p, axis=0)
        return carry

    lax.fori_loop(0, H, head_body, 0)
    for cp in late_copies:
        cp.wait()
    finalize(H - 1, NQB - 1, weigh(H - 1, NKC - 1, NQB - 1, _blocks(p_v[...])))
    for qb in range(NQB - 1):
        finalize(H - 1, qb, fin_v[qb][...])
    safe = (st_v[0] >= SUM_LO) & (st_v[1] <= SUM_HI) & (jnp.abs(st_v[2]) <= F32_MAX)
    unsafe = jnp.sum(jnp.where(safe, 0.0, 1.0)) != 0.0

    wr = wr_ref[...].astype(F32).reshape(1, D)

    def residual(i):
        rows = slice(i * RES_ROWS, (i + 1) * RES_ROWS)
        return x_v[rows, :].astype(F32) + lax.dot_general(
            _unpack(ot_v[:, rows]), wo_v[...], TN, preferred_element_type=F32)

    def project_and_route():
        packed = [jnp.full((8, 128), -F32_MAX, F32) for _ in range(S // 1024)]
        last_keys = []
        ahead = [residual(0), residual(1)]
        for i in range(S // RES_ROWS):
            if i + 2 < S // RES_ROWS:
                ahead.append(residual(i + 2))
            hh = ahead.pop(0)
            cen, rstd = _center(hh)
            r = jnp.sum(cen * wr, axis=-1, keepdims=True) * rstd
            ln = cen * rstd
            res = hh + ln
            rows = slice(i * RES_ROWS, (i + 1) * RES_ROWS)
            ln_v[rows, :] = ln
            res_v[rows, :] = res
            out_v[rows, :] = res.astype(BF16)
            for cp, lo, n in zip(out_copies, OUT_LO, OUT_ROWS):
                if lo + n == rows.stop:
                    cp.start()
            for g, rg in enumerate(_blocks(r), rows.start // 8):
                if g * 8 < OUT_LO[-1]:
                    packed[g // 128] = jnp.where(lane == g % 128, rg, packed[g // 128])
                else:
                    last_keys.append(_router_key(rg, sub[:, 0:1] + g * 8))

        keys = [_router_key(v, (lane + 128 * j) * 8 + sub) for j, v in enumerate(packed)]
        top1 = jnp.max(jnp.maximum(*keys), axis=1, keepdims=True)
        keys = [jnp.where(k == top1, -jnp.inf, k) for k in keys]
        top2 = jnp.max(jnp.maximum(*keys), axis=1, keepdims=True)
        for key in last_keys:
            top2 = jnp.maximum(top2, jnp.minimum(top1, key))
            top1 = jnp.maximum(top1, key)
        for w in (4, 2, 1):
            o1, o2 = pltpu.roll(top1, w, 0), pltpu.roll(top2, w, 0)
            top2 = jnp.maximum(jnp.maximum(top2, o2), jnp.minimum(top1, o1))
            top1 = jnp.maximum(top1, o1)
        for n, key in enumerate((top1, top2)):
            idx_s[n] = (~pltpu.bitcast(key, jnp.int32) & (S - 1))[0, 0]

    project_and_route()

    @pl.when(unsafe)
    def _():
        def k_rows(i, carry):
            rows = pl.ds(pl.multiple_of(i * 128, 128), 128)
            xn = _layernorm(x_v[rows, :].astype(F32)).astype(BF16)
            res_v[rows, :] = jnp.dot(xn, wk_v[...], preferred_element_type=F32)
            return carry

        def one_head(h, carry):
            ln_v[:, 0:128] = _to_front(res_v[:, pl.ds(pl.multiple_of((h >> 3) * 128, 128), 128)], h)

            def one_block(qb, carry):
                cols = pl.ds(pl.multiple_of(qb * BQ, BQ), BQ)
                s = jnp.dot(ln_v[:, 0:DH], qt_v[_head_rows(h), cols], preferred_element_type=F32)
                p = jnp.exp2(s - jnp.max(s, axis=0, keepdims=True))
                p = p * (1.0 / jnp.sum(p, axis=0, keepdims=True))
                ot_v[_head_pairs(h), cols] = _pack(
                    jnp.dot(_unpack(vt_v[_head_pairs(h), :]), p, preferred_element_type=F32))
                return carry

            return lax.fori_loop(0, NQB, one_block, carry)

        lax.fori_loop(0, S // 128, k_rows, 0)
        lax.fori_loop(0, H, one_head, 0)
        for cp in out_copies:
            cp.wait()
        project_and_route()

    i1, i2 = idx_s[0], idx_s[1]
    row = lax.broadcasted_iota(jnp.int32, (16, D), 0)
    xs = jnp.where(row < 8, ln_v[pl.ds(i1, 1), :], ln_v[pl.ds(i2, 1), :])
    hs = jnp.where(row < 8, res_v[pl.ds(i1, 1), :], res_v[pl.ds(i2, 1), :])
    gate = jax.nn.sigmoid(jnp.sum(xs * wr, axis=-1, keepdims=True))
    xs = xs.astype(BF16)
    gg = jnp.dot(xs, wg_v[...], preferred_element_type=F32)
    uu = jnp.dot(xs, wu_v[...], preferred_element_type=F32)
    act = (gg * jax.nn.sigmoid(gg) * uu).astype(BF16)
    routed = hs + jnp.dot(act, wd_v[...], preferred_element_type=F32) * gate

    for cp in out_copies:
        cp.wait()
    patches = []
    for n, i in enumerate((i1, i2)):
        rows = pl.ds(pl.multiple_of((i >> 4) * 16, 16), 16)
        out_v[rows, :] = jnp.where(row == i & 15, routed[8 * n:8 * n + 1], out_v[rows, :].astype(F32)).astype(BF16)
        patches.append(pltpu.make_async_copy(out_v.at[rows, :], out_hbm.at[0, rows, :], f_sem.at[n]))
    patches[0].start()

    @pl.when(i1 >> 4 != i2 >> 4)
    def _():
        patches[1].start()
        patches[1].wait()

    patches[0].wait()


@jax.jit
def pallas_sequential_preLN__mha_block__moe_arch_mod__prompt_kernel(
    A_x: jax.Array,
    A_wqkv: jax.Array,
    A_wo: jax.Array,
    B_x: jax.Array,
    B_w_r: jax.Array,
    B_w_gate: jax.Array,
    B_w_up: jax.Array,
    B_w_down: jax.Array,
):
    del B_x
    hbm = pl.BlockSpec(memory_space=pltpu.HBM)
    return pl.pallas_call(
        _kernel,
        out_shape=jax.ShapeDtypeStruct((1, S, D), BF16),
        in_specs=[hbm, hbm, hbm, pl.BlockSpec(memory_space=pltpu.VMEM), hbm, hbm, hbm],
        out_specs=hbm,
        scratch_shapes=[
            pltpu.VMEM((S, D), BF16),
            pltpu.VMEM((D, D), BF16),
            pltpu.VMEM((D, D), BF16),
            pltpu.VMEM((D, D), BF16),
            pltpu.VMEM((D, D), BF16),
            pltpu.VMEM((D, FF), BF16),
            pltpu.VMEM((D, FF), BF16),
            pltpu.VMEM((FF, D), BF16),
            pltpu.VMEM((7, S // 4, D // 2), U32),
            pltpu.VMEM((3, 7, D // 4, D // 2), U32),
            pltpu.VMEM((D // 128, MXU_KEYS, 128), F32),
            pltpu.VMEM((VPU_KEYS_PAD, D), F32),
            pltpu.VMEM((H, 2, VPU_KEYS_PAD, 128), F32),
            pltpu.VMEM((D, S), F32),
            pltpu.VMEM((D, S), F32),
            pltpu.VMEM((D // 2, S), U32),
            pltpu.VMEM((D // 2, S), U32),
            pltpu.VMEM((S, D), F32),
            pltpu.VMEM((S, D), F32),
            pltpu.VMEM((S, D), BF16),
            pltpu.VMEM((MXU_KEYS, 128), F32),
            pltpu.VMEM((2 * DH, S), F32),
            pltpu.VMEM((DH, S), F32),
            pltpu.VMEM((DH, S), F32),
            [pltpu.VMEM((BK, 128), F32)] * NKC,
            [pltpu.VMEM((len(v) * DH * 8, 128), F32) for v in VPU_BLOCKS],
            pltpu.VMEM((BK, BQ), F32),
            [pltpu.VMEM((EARLY * 8, BQ), F32)] * NQB,
            [pltpu.VMEM((DH + 8, BQ), F32)] * NQB,
            [pltpu.VMEM((DH + 8, BQ), F32)] * NQB,
            pltpu.VMEM((3, 8, S), F32),
            pltpu.SMEM((2,), jnp.int32),
            pltpu.SemaphoreType.DMA((len(X_ROWS),)),
            pltpu.SemaphoreType.DMA((7,)),
            pltpu.SemaphoreType.DMA((len(OUT_ROWS),)),
            pltpu.SemaphoreType.DMA((2,)),
        ],
        compiler_params=pltpu.CompilerParams(vmem_limit_bytes=100 * 2 ** 20),
    )(A_x, A_wqkv, A_wo, B_w_r, B_w_gate, B_w_up, B_w_down)
```

```python
import math

import jax
import jax.numpy as jnp
from jax import lax
from jax.experimental import pallas as pl
from jax.experimental.pallas import tpu as pltpu

F32 = jnp.float32
BF16 = jnp.bfloat16
U32 = jnp.uint32

S = 2048
D = 512
H = 32
DH = 16
FF = 1792
EPS = 1e-5
QSCALE = DH ** -0.5 * math.log2(math.e)

BK = 128
BQ = 512
NKC = S // BK
NQB = S // BQ
NBLK = BK // 8
NLT = BQ // 128

VPU_FIXED = [0, 7]
VPU_EXTRA = 12
_NONE, _ONE, _TWO = ["0000"] * 4, ["1000", "0100", "0010", "0001"], ["1100", "0011"] * 2
EXTRA_TILES = [_NONE, _TWO, _ONE] + [_TWO] * 12 + [_ONE]
VPU_BLOCKS = [VPU_FIXED + ([VPU_EXTRA] if "1" in "".join(x) else []) for x in EXTRA_TILES]
MXU_BLOCKS = [b for b in range(NBLK - 1, -1, -1) if b not in VPU_FIXED]
NM = len(MXU_BLOCKS)
EARLY = 2
NEW_SUMS = 2
LATE_Q = NKC - 4

PROJ_ORDER = ("w0 L0 wk fk K0 wq w1 fq L2 Q0 L1 K2 K1 wv w2 late Q1 L3 Q2 K3 Q3 L4 K4 B0 L5 K5 Q4 L6 fv "
              "Q6 Q5 K6 V3 B1 B2 V1 V0 V2 V4 V6 V5").split()
X_ROWS = [512, 512, 1024]
PROJ_ROWS = [512] + [256] * 6
OUT_ROWS = [1280, 512, 256]
RES_ROWS = 128

SUM_LO = 2.0 ** -80
SUM_HI = 2.0 ** 120
F32_MAX = 3.0e38
TINY = 2.0 ** -100

TN = (((0,), (0,)), ((), ()))
NT = (((1,), (1,)), ((), ()))


def _starts(sizes):
    return [sum(sizes[:i]) for i in range(len(sizes))]


X_LO, PROJ_LO, OUT_LO = _starts(X_ROWS), _starts(PROJ_ROWS), _starts(OUT_ROWS)
VPU_LO = _starts([8 * len(v) for v in VPU_BLOCKS])
VPU_KEYS = VPU_LO[-1] + 8 * len(VPU_BLOCKS[-1])
VPU_KEYS_PAD = -(-VPU_KEYS // 128) * 128
MXU_KEYS = NKC * NM * 8


def _mxu_row(c, b):
    return (c * NM + MXU_BLOCKS.index(b) - EARLY) * 8 % MXU_KEYS


def _moments(v):
    mean = jnp.sum(v, axis=-1, keepdims=True) * (1.0 / D)
    c = v - mean
    return mean, c, lax.rsqrt(jnp.sum(c * c, axis=-1, keepdims=True) * (1.0 / D) + EPS)


def _layernorm(v):
    _, c, rstd = _moments(v)
    return c * rstd


def _pack(v):
    return pltpu.bitcast(v.astype(BF16), U32)


def _unpack(v):
    return pltpu.bitcast(v, BF16)


def _quadrants(v):
    m, n = v.shape[0] // 2, v.shape[1] // 2
    return v[:m, :n], v[:m, n:], v[m:, :n], v[m:, n:]


def _blocks(v):
    return [v[r:r + 8] for r in range(0, v.shape[0], 8)]


def _head_rows(h):
    return pl.ds(pl.multiple_of(h * DH, DH), DH)


def _head_pairs(h):
    return pl.ds(pl.multiple_of(h * (DH // 2), DH // 2), DH // 2)


def _to_front(v, h):
    return pltpu.roll(v, (128 - (h & 7) * DH) & 127, 1)


def _router_key(r, tok):
    r = jnp.clip(r + TINY, -F32_MAX, F32_MAX)
    return pltpu.bitcast((pltpu.bitcast(r, jnp.int32) | (S - 1)) ^ tok, F32)


def _kernel(x_hbm, wqkv_hbm, wo_hbm, wr_hbm, wg_hbm, wu_hbm, wd_hbm, out_hbm,
            x_v, wq_v, wk_v, wv_v, wo_v, wg_v, wu_v, wd_v,
            xf_v, wf_v, km_v, kv_v, base_v, qt_v, qk_v, vt_v, ot_v, res_v, ln_v, out_v,
            qm_v, qs_v, qa_v, lhs_v, kb_v, p_v, early_v, acc_v, fin_v, st_v, routed_v, wr_v, idx_s,
            x_sem, w_sem, o_sem, f_sem):
    lane = lax.broadcasted_iota(jnp.int32, (8, 128), 1)
    sub = lax.broadcasted_iota(jnp.int32, (8, 128), 0)

    first_copies = {
        "q": pltpu.make_async_copy(wqkv_hbm.at[:, pl.ds(0, D)], wq_v, w_sem.at[0]),
        "k": pltpu.make_async_copy(wqkv_hbm.at[:, pl.ds(D, D)], wk_v, w_sem.at[1]),
        "v": pltpu.make_async_copy(wqkv_hbm.at[:, pl.ds(2 * D, D)], wv_v, w_sem.at[2]),
    }
    for i, (lo, n) in enumerate(zip(X_LO, X_ROWS)):
        first_copies[str(i)] = pltpu.make_async_copy(
            x_hbm.at[0, pl.ds(lo, n), :], x_v.at[pl.ds(lo, n), :], x_sem.at[i])
    late_copies = [
        pltpu.make_async_copy(wo_hbm, wo_v, w_sem.at[3]),
        pltpu.make_async_copy(wg_hbm, wg_v, w_sem.at[4]),
        pltpu.make_async_copy(wu_hbm, wu_v, w_sem.at[5]),
        pltpu.make_async_copy(wd_hbm, wd_v, w_sem.at[6]),
        pltpu.make_async_copy(wr_hbm, wr_v, w_sem.at[7]),
    ]
    out_copies = [
        pltpu.make_async_copy(out_v.at[pl.ds(lo, n), :], out_hbm.at[0, pl.ds(lo, n), :], o_sem.at[i])
        for i, (lo, n) in enumerate(zip(OUT_LO, OUT_ROWS))
    ]

    def ln1(i):
        half = PROJ_ROWS[i] // 2
        for r in range(0, half, 128):
            top, bot = PROJ_LO[i] + r, PROJ_LO[i] + half + r
            xx = jnp.concatenate([x_v[top:top + 128, :], x_v[bot:bot + 128, :]], axis=0)
            a11, a12, a21, a22 = _quadrants(_layernorm(xx.astype(F32)))
            lo = (PROJ_LO[i] // 2 + r) // 2
            for n, v in enumerate((a21 + a22, a11 + a12, a11, a22, a11 + a22, a21 - a11, a12 - a22)):
                xf_v[n, lo:lo + 64, :] = _pack(v)

    def w_factors(name):
        w_v, n = {"k": (wk_v, 0), "q": (wq_v, 1), "v": (wv_v, 2)}[name]
        b11, b12, b21, b22 = _quadrants(w_v[...].astype(F32))
        for j, v in enumerate((b11, b22, b12 - b22, b21 - b11, b11 + b22, b11 + b12, b21 + b22)):
            wf_v[n, j] = _pack(v.T if name == "v" else v)

    def project(i, n, transpose):
        m = []
        for j in range(7):
            xf = _unpack(xf_v[j, PROJ_LO[i] // 4:(PROJ_LO[i] + PROJ_ROWS[i]) // 4, :])
            wf = _unpack(wf_v[n, j])
            if transpose:
                m.append(lax.dot_general(wf, xf, NT, preferred_element_type=F32))
            else:
                m.append(jnp.dot(xf, wf, preferred_element_type=F32))
        m2, m5, m3, m4, m1, m6, m7 = m
        c11, c12, c21, c22 = (m4 - m5 + m1) + m7, m5 + m3, m2 + m4, (m3 - m2 + m1) + m6
        if transpose:
            c12, c21 = c21, c12
        return jnp.concatenate([jnp.concatenate([c11, c12], axis=1), jnp.concatenate([c21, c22], axis=1)], axis=0)

    def proj_k(i):
        kk = _blocks(project(i, 0, False))
        for t in range(PROJ_ROWS[i] // BK):
            c = PROJ_LO[i] // BK + t
            for part in (MXU_BLOCKS[:EARLY], MXU_BLOCKS[EARLY:]):
                v = jnp.concatenate([kk[t * NBLK + b] for b in part], axis=0)
                rows = slice(_mxu_row(c, part[0]), _mxu_row(c, part[0]) + v.shape[0])
                for n in range(D // 128):
                    km_v[n, rows, :] = v[:, n * 128:(n + 1) * 128]
            v = jnp.concatenate([kk[t * NBLK + b] for b in VPU_BLOCKS[c]], axis=0)
            kv_v[VPU_LO[c]:VPU_LO[c] + v.shape[0], :] = v

    def proj_q(i):
        qq = (project(i, 1, False) * QSCALE).T
        qt_v[:, PROJ_LO[i]:PROJ_LO[i] + PROJ_ROWS[i]] = qq
        skew = (lane + sub) & 7
        for t in range(0, PROJ_ROWS[i], 128):
            tile = [jnp.take_along_axis(b, skew, axis=0) for b in _blocks(qq[:, t:t + 128])]
            qk_v[:, PROJ_LO[i] + t:PROJ_LO[i] + t + 128] = jnp.concatenate(tile, axis=0)

    def proj_v(i):
        vt_v[:, PROJ_LO[i]:PROJ_LO[i] + PROJ_ROWS[i]] = _pack(project(i, 2, True))

    def k_bases(n):
        if (n + 1) * 128 > VPU_KEYS:
            kv_v[VPU_KEYS:, :] = jnp.zeros((VPU_KEYS_PAD - VPU_KEYS, D), F32)
        for r, b in enumerate(_blocks(kv_v[n * 128:(n + 1) * 128, :].T)):
            base_v[r // 2, r % 2, n * 128:(n + 1) * 128, :] = jnp.concatenate([b] * 16, axis=0).T

    for n in PROJ_ORDER:
        if n[0] == "w":
            first_copies[n[1]].start()
    for n in PROJ_ORDER:
        if n == "late":
            for cp in late_copies:
                cp.start()
        elif n[0] == "w":
            first_copies[n[1]].wait()
        elif n[0] == "f":
            w_factors(n[1])
        else:
            {"L": ln1, "K": proj_k, "Q": proj_q, "V": proj_v, "B": k_bases}[n[0]](int(n[1]))

    def stage_keys(h, c, step):
        own = NM - EARLY if c == NKC - 1 else NM
        rows = slice(VPU_LO[c], VPU_LO[c] + 8 * len(VPU_BLOCKS[c]))
        turns = [jnp.concatenate([base_v[h, 0, rows, :], base_v[h, 1, rows, :]], axis=0)]
        for r in range(8):
            if r > step:
                turns.append(pltpu.roll(turns[r - step], 128 - step, 1))
            elif r:
                turns.append(pltpu.roll(turns[0], 128 - r, 1))
            if r < 7:
                lo, hi = own * r // 7 * 8, own * (r + 1) // 7 * 8
                lhs_v[c][lo:hi, :] = _to_front(km_v[h >> 3, c * NM * 8 + lo:c * NM * 8 + hi, :], h)
        if own < NM:
            h2 = jnp.minimum(h + 1, H - 1)
            lhs_v[c][own * 8:NM * 8, :] = _to_front(km_v[h2 >> 3, MXU_KEYS - EARLY * 8:, :], h2)
        kb_v[c][...] = jnp.concatenate(turns, axis=0)

    def probs(c, qb):
        by_blk = dict(zip(MXU_BLOCKS[:EARLY], _blocks(early_v[qb][...])))
        lhs = _blocks(lhs_v[c][0:NM * 8, 0:DH])
        q_v = qa_v if c >= LATE_Q else qs_v
        last = c == NKC - 1
        tiles = []
        for t in range(NLT):
            cols = slice(qb * BQ + t * 128, qb * BQ + (t + 1) * 128)
            on_vpu = VPU_FIXED + ([VPU_EXTRA] if EXTRA_TILES[c][qb][t] == "1" else [])
            names = MXU_BLOCKS[EARLY:] + ([] if last else [None] * EARLY)
            take = [j for j, b in enumerate(names) if b not in on_vpu]
            e = jnp.exp2(jnp.dot(jnp.concatenate([lhs[j] for j in take], axis=0), qm_v[0:DH, cols],
                                 preferred_element_type=F32))
            tile = {names[j]: v for j, v in zip(take, _blocks(e)) if names[j] is not None}
            if not last:
                early_v[qb][:, t * 128:(t + 1) * 128] = e[-EARLY * 8:]
            s = None
            for d in range(DH):
                lo = (d % 8 * 2 + d // 8) * len(VPU_BLOCKS[c]) * 8
                term = kb_v[c][lo:lo + len(on_vpu) * 8, :] * q_v[d:d + 1, cols]
                s = term if d == 0 else s + term
            tile.update(zip(on_vpu, _blocks(jnp.exp2(s))))
            tiles.append(tile)
        if last:
            early_v[qb][...] = jnp.exp2(jnp.dot(
                jnp.concatenate(lhs[-EARLY:], axis=0), qm_v[DH:2 * DH, qb * BQ:(qb + 1) * BQ],
                preferred_element_type=F32))
        by_blk.update({b: jnp.concatenate([tile[b] for tile in tiles], axis=1) for b in tiles[0]})
        return [by_blk[b] for b in range(NBLK - 1, -1, -1)]

    def sums_after(c):
        return fin_v if c >= NEW_SUMS else acc_v

    def weigh(h, c, qb, p):
        o = jnp.dot(_unpack(vt_v[_head_pairs(h), c * BK:(c + 1) * BK]), jnp.concatenate(p[::-1], axis=0),
                    preferred_element_type=F32)
        terms = p[2:14] + [p[0]] + p[14:] + [p[1]]
        if c > 0:
            old = sums_after(c - 1)[qb][...]
            o = old[0:DH] + o
            terms.append(old[DH:])
        l = terms[0]
        for v in terms[1:]:
            l = l + v
        return jnp.concatenate([o, l], axis=0)

    def finalize(h, qb, sums):
        l = jnp.sum(sums[DH:], axis=0, keepdims=True)
        r = pltpu.reciprocal(l, approx=True)
        o = sums[0:DH] * (r * (2.0 - l * r))
        cols = slice(qb * BQ, (qb + 1) * BQ)
        ot_v[_head_pairs(h), cols] = _pack(o)
        st_v[0, 0:1, cols] = jnp.minimum(st_v[0, 0:1, cols], l)
        st_v[1, 0:1, cols] = jnp.maximum(st_v[1, 0:1, cols], l)

    for c in range(NKC):
        stage_keys(0, c, 8)
    qm_v[0:DH, :] = qt_v[0:DH, :]
    qs_v[...] = qk_v[0:DH, :]
    first = jnp.exp2(jnp.dot(km_v[0, MXU_KEYS - EARLY * 8:, 0:DH], qt_v[0:DH, :], preferred_element_type=F32))
    for qb in range(NQB):
        early_v[qb][...] = first[:, qb * BQ:(qb + 1) * BQ]
    p_v[...] = jnp.zeros(p_v.shape, F32)
    for ref in (*fin_v, st_v):
        ref[...] = jnp.ones(ref.shape, F32)

    def head_body(h, carry):
        prv = jnp.maximum(h - 1, 0)
        nxt = jnp.minimum(h + 1, H - 1)

        p, (ph, pc, pq) = _blocks(p_v[...]), (prv, NKC - 1, NQB - 1)
        for c in range(NKC):
            for qb in range(NQB):
                p_next = probs(c, qb)
                sums = weigh(ph, pc, pq, p)
                if pc == NEW_SUMS:
                    finalize(prv, pq, fin_v[pq][...])
                sums_after(pc)[pq][...] = sums
                p, (ph, pc, pq) = p_next, (h, c, qb)
            stage_keys(nxt, c, 2)
            if c == 1:
                qa_v[...] = qs_v[...]
                qm_v[DH:2 * DH, :] = qt_v[_head_rows(nxt), :]
        qm_v[0:DH, :] = qm_v[DH:2 * DH, :]
        qs_v[...] = qk_v[_head_rows(nxt), :]
        p_v[...] = jnp.concatenate(p, axis=0)
        return carry

    lax.fori_loop(0, H, head_body, 0)
    for cp in late_copies:
        cp.wait()
    finalize(H - 1, NQB - 1, weigh(H - 1, NKC - 1, NQB - 1, _blocks(p_v[...])))
    for qb in range(NQB - 1):
        finalize(H - 1, qb, fin_v[qb][...])
    outside = jnp.sum(jnp.where((st_v[0] >= SUM_LO) & (st_v[1] <= SUM_HI), 0.0, 1.0))

    wr = wr_v[...].astype(F32).reshape(1, D)
    row = lax.broadcasted_iota(jnp.int32, (16, D), 0)

    def residual(i):
        rows = slice(i * RES_ROWS, (i + 1) * RES_ROWS)
        return x_v[rows, :].astype(F32) + lax.dot_general(
            _unpack(ot_v[:, rows]), wo_v[...], TN, preferred_element_type=F32)

    def second_half():
        packed = [jnp.full((8, 128), -F32_MAX, F32) for _ in range(S // 1024)]
        last_keys = []
        total = jnp.zeros((8, 1), F32)
        ahead = [residual(0), residual(1)]
        for i in range(S // RES_ROWS):
            if i + 2 < S // RES_ROWS:
                ahead.append(residual(i + 2))
            hh = ahead.pop(0)
            mean, cen, rstd = _moments(hh)
            for v in _blocks(mean):
                total = total + v
            r = jnp.sum(cen * wr, axis=-1, keepdims=True) * rstd
            ln = cen * rstd
            res = hh + ln
            rows = slice(i * RES_ROWS, (i + 1) * RES_ROWS)
            ln_v[rows, :] = ln
            res_v[rows, :] = res
            out_v[rows, :] = res.astype(BF16)
            for cp, lo, n in zip(out_copies, OUT_LO, OUT_ROWS):
                if lo + n == rows.stop:
                    cp.start()
            for g, rg in enumerate(_blocks(r), rows.start // 8):
                if g * 8 < OUT_LO[-1]:
                    packed[g // 128] = jnp.where(lane == g % 128, rg, packed[g // 128])
                else:
                    last_keys.append(_router_key(rg, sub[:, 0:1] + g * 8))

        keys = [_router_key(v, (lane + 128 * j) * 8 + sub) for j, v in enumerate(packed)]
        top1 = jnp.max(jnp.maximum(*keys), axis=1, keepdims=True)
        keys = [jnp.where(k == top1, -jnp.inf, k) for k in keys]
        top2 = jnp.max(jnp.maximum(*keys), axis=1, keepdims=True)
        for key in last_keys:
            top2 = jnp.maximum(top2, jnp.minimum(top1, key))
            top1 = jnp.maximum(top1, key)
        for w in (4, 2, 1):
            o1, o2 = pltpu.roll(top1, w, 0), pltpu.roll(top2, w, 0)
            top2 = jnp.maximum(jnp.maximum(top2, o2), jnp.minimum(top1, o1))
            top1 = jnp.maximum(top1, o1)
        i1, i2 = ((~pltpu.bitcast(key, jnp.int32) & (S - 1))[0, 0] for key in (top1, top2))
        idx_s[0] = i1
        idx_s[1] = i2

        xs = jnp.where(row < 8, ln_v[pl.ds(i1, 1), :], ln_v[pl.ds(i2, 1), :])
        hs = jnp.where(row < 8, res_v[pl.ds(i1, 1), :], res_v[pl.ds(i2, 1), :])
        gate = jax.nn.sigmoid(jnp.sum(xs * wr, axis=-1, keepdims=True))
        xs = xs.astype(BF16)
        gg = jnp.dot(xs, wg_v[...], preferred_element_type=F32)
        uu = jnp.dot(xs, wu_v[...], preferred_element_type=F32)
        act = (gg * jax.nn.sigmoid(gg) * uu).astype(BF16)
        routed_v[...] = hs + jnp.dot(act, wd_v[...], preferred_element_type=F32) * gate
        return total

    total = second_half()
    for w in (4, 2, 1):
        total = total + pltpu.roll(total, w, 0)
    overflowed = jnp.where(jnp.abs(total) <= F32_MAX, 0, 1)[0, 0]

    @pl.when((outside != 0.0) | (overflowed != 0))
    def _():
        def k_rows(i, carry):
            rows = pl.ds(pl.multiple_of(i * 128, 128), 128)
            xn = _layernorm(x_v[rows, :].astype(F32)).astype(BF16)
            res_v[rows, :] = jnp.dot(xn, wk_v[...], preferred_element_type=F32)
            return carry

        def one_head(h, carry):
            ln_v[:, 0:128] = _to_front(res_v[:, pl.ds(pl.multiple_of((h >> 3) * 128, 128), 128)], h)

            def one_block(qb, carry):
                cols = pl.ds(pl.multiple_of(qb * BQ, BQ), BQ)
                s = jnp.dot(ln_v[:, 0:DH], qt_v[_head_rows(h), cols], preferred_element_type=F32)
                p = jnp.exp2(s - jnp.max(s, axis=0, keepdims=True))
                p = p * (1.0 / jnp.sum(p, axis=0, keepdims=True))
                ot_v[_head_pairs(h), cols] = _pack(
                    jnp.dot(_unpack(vt_v[_head_pairs(h), :]), p, preferred_element_type=F32))
                return carry

            return lax.fori_loop(0, NQB, one_block, carry)

        lax.fori_loop(0, S // 128, k_rows, 0)
        lax.fori_loop(0, H, one_head, 0)
        for cp in out_copies:
            cp.wait()
        second_half()

    i1, i2 = idx_s[0], idx_s[1]
    for cp in out_copies:
        cp.wait()
    patches = []
    for n, i in enumerate((i1, i2)):
        rows = pl.ds(pl.multiple_of((i >> 4) * 16, 16), 16)
        old = out_v[rows, :].astype(F32)
        out_v[rows, :] = jnp.where(row == i & 15, routed_v[8 * n:8 * n + 1, :], old).astype(BF16)
        patches.append(pltpu.make_async_copy(out_v.at[rows, :], out_hbm.at[0, rows, :], f_sem.at[n]))
    patches[0].start()

    @pl.when(i1 >> 4 != i2 >> 4)
    def _():
        patches[1].start()
        patches[1].wait()

    patches[0].wait()


@jax.jit
def pallas_sequential_preLN__mha_block__moe_arch_mod__prompt_kernel(
    A_x: jax.Array,
    A_wqkv: jax.Array,
    A_wo: jax.Array,
    B_x: jax.Array,
    B_w_r: jax.Array,
    B_w_gate: jax.Array,
    B_w_up: jax.Array,
    B_w_down: jax.Array,
):
    del B_x
    hbm = pl.BlockSpec(memory_space=pltpu.HBM)
    return pl.pallas_call(
        _kernel,
        out_shape=jax.ShapeDtypeStruct((1, S, D), BF16),
        in_specs=[hbm] * 7,
        out_specs=hbm,
        scratch_shapes=[
            pltpu.VMEM((S, D), BF16),
            pltpu.VMEM((D, D), BF16),
            pltpu.VMEM((D, D), BF16),
            pltpu.VMEM((D, D), BF16),
            pltpu.VMEM((D, D), BF16),
            pltpu.VMEM((D, FF), BF16),
            pltpu.VMEM((D, FF), BF16),
            pltpu.VMEM((FF, D), BF16),
            pltpu.VMEM((7, S // 4, D // 2), U32),
            pltpu.VMEM((3, 7, D // 4, D // 2), U32),
            pltpu.VMEM((D // 128, MXU_KEYS, 128), F32),
            pltpu.VMEM((VPU_KEYS_PAD, D), F32),
            pltpu.VMEM((H, 2, VPU_KEYS_PAD, 128), F32),
            pltpu.VMEM((D, S), F32),
            pltpu.VMEM((D, S), F32),
            pltpu.VMEM((D // 2, S), U32),
            pltpu.VMEM((D // 2, S), U32),
            pltpu.VMEM((S, D), F32),
            pltpu.VMEM((S, D), F32),
            pltpu.VMEM((S, D), BF16),
            pltpu.VMEM((2 * DH, S), F32),
            pltpu.VMEM((DH, S), F32),
            pltpu.VMEM((DH, S), F32),
            [pltpu.VMEM((BK, 128), F32)] * NKC,
            [pltpu.VMEM((len(v) * DH * 8, 128), F32) for v in VPU_BLOCKS],
            pltpu.VMEM((BK, BQ), F32),
            [pltpu.VMEM((EARLY * 8, BQ), F32)] * NQB,
            [pltpu.VMEM((DH + 8, BQ), F32)] * NQB,
            [pltpu.VMEM((DH + 8, BQ), F32)] * NQB,
            pltpu.VMEM((2, 8, S), F32),
            pltpu.VMEM((16, D), F32),
            pltpu.VMEM((D,), BF16),
            pltpu.SMEM((2,), jnp.int32),
            pltpu.SemaphoreType.DMA((len(X_ROWS),)),
            pltpu.SemaphoreType.DMA((8,)),
            pltpu.SemaphoreType.DMA((len(OUT_ROWS),)),
            pltpu.SemaphoreType.DMA((2,)),
        ],
        compiler_params=pltpu.CompilerParams(vmem_limit_bytes=100 * 2 ** 20),
    )(A_x, A_wqkv, A_wo, B_w_r, B_w_gate, B_w_up, B_w_down)
```
